```python
import jax
import jax.numpy as jnp

def _softmax(x, axis=-1):
    return jax.nn.softmax(x, axis=axis)
def _gelu(x):
    return jax.nn.gelu(x, approximate=True)
def _silu(x):
    return jax.nn.silu(x)
def _sigmoid(x):
    return jax.nn.sigmoid(x)
def _layernorm(x, axis=-1, eps=1e-5):
    m = jnp.mean(x, axis=axis, keepdims=True)
    v = jnp.var(x, axis=axis, keepdims=True)
    return (x - m) / jnp.sqrt(v + eps)
def _scatter_add(tgt, idx, src, axis=0):
    return tgt.at[idx].add(src)
def _segment_sum(src, seg, n):
    return jax.ops.segment_sum(src, seg, n)
class _Rng:
    def __init__(self, key):
        self._k = key
    def _next(self):
        self._k, sub = jax.random.split(self._k)
        return sub
    def normal(self, shape):
        return jax.random.normal(self._next(), shape, dtype=jnp.bfloat16)
    def randint(self, lo, hi, shape):
        return jax.random.randint(self._next(), shape, lo, hi, dtype=jnp.int32)
    def uniform(self, shape, lo=0.0, hi=1.0):
        return jax.random.uniform(self._next(), shape, jnp.bfloat16, lo, hi)
    def permutation(self, n):
        return jax.random.permutation(self._next(), n)


kernel_name = 'recurrent_scan__compressed_kv_cla__moe_arch_mod__decode'

def setup_inputs():
    _rng = _Rng(jax.random.key(int.from_bytes(__import__("os").urandom(4), "little")))
    _w = (lambda a: (lambda t: t.astype(jnp.bfloat16) if jnp.issubdtype(t.dtype, jnp.floating) else t)(jnp.asarray(a)))
    def _A_setup():
        B, H, Sq, Sk, D, M = 4, 32, 1, 4096, 128, 576
        Dc = 4 * D
        return {
            "x": _w((lambda *s: _rng.normal(s) * 0.05)(B, Sq, M)),
            "c_kv": _w((lambda *s: _rng.normal(s) * 0.05)(B, Sk, Dc)),
            "w_q": _w((lambda *s: _rng.normal(s) * 0.05)(M, H, D) * (M ** -0.5)),
            "w_uk": _w((lambda *s: _rng.normal(s) * 0.05)(Dc, H, D) * (Dc ** -0.5)),
            "w_uv": _w((lambda *s: _rng.normal(s) * 0.05)(Dc, H, D) * (Dc ** -0.5)),
            "w_o": _w((lambda *s: _rng.normal(s) * 0.05)(H, D, M) * ((H * D) ** -0.5)),
        }
    _A_in = _A_setup()

    def _B_setup():
        B, S, D, F, C = 4, 1, 576, 4608, 1
        return {
            "x": _w((lambda *s: _rng.normal(s) * 0.05)(B, S, D)),
            "w_r": _w((lambda *s: _rng.normal(s) * 0.05)(D)),
            "w_gate": _w((lambda *s: _rng.normal(s) * 0.05)(D, F)),
            "w_up": _w((lambda *s: _rng.normal(s) * 0.05)(D, F)),
            "w_down": _w((lambda *s: _rng.normal(s) * 0.05)(F, D)),
        }
    _B_in = _B_setup()

    return {
        "A_x": _A_in["x"],
        "A_c_kv": _A_in["c_kv"],
        "A_w_q": _A_in["w_q"],
        "A_w_uk": _A_in["w_uk"],
        "A_w_uv": _A_in["w_uv"],
        "A_w_o": _A_in["w_o"],
        "B_x": _B_in["x"],
        "B_w_r": _B_in["w_r"],
        "B_w_gate": _B_in["w_gate"],
        "B_w_up": _B_in["w_up"],
        "B_w_down": _B_in["w_down"],
    }

def reference(A_x, A_c_kv, A_w_q, A_w_uk, A_w_uv, A_w_o, B_x, B_w_r, B_w_gate, B_w_up, B_w_down):
    def _A_ref(x, c_kv, w_q, w_uk, w_uv, w_o):
        B, Sq, M = x.shape[0], x.shape[1], x.shape[2]
        Sk = c_kv.shape[1]
        H, D = w_q.shape[1], w_q.shape[2]
        q = jnp.einsum("bqm,mhd->bhqd", x, w_q)
        k = jnp.einsum("bkc,chd->bhkd", c_kv, w_uk)
        v = jnp.einsum("bkc,chd->bhkd", c_kv, w_uv)
        scores = jnp.einsum("bhqd,bhkd->bhqk", q, k) * (D ** -0.5)
        off = Sk - Sq
        qi = jnp.arange(Sq)[:, None]
        kj = jnp.arange(Sk)[None, :]
        cmask = kj <= (qi + off)
        scores = jnp.where(cmask[None, None], scores, -1e9)
        p = _softmax(scores, axis=-1)
        ctx = jnp.einsum("bhqk,bhkd->bhqd", p, v)
        return jnp.einsum("bhqd,hdm->bqm", ctx, w_o)

    def _B_ref(x, w_r, w_gate, w_up, w_down):
        B, S, D = x.shape
        C = 1
        r = x @ w_r
        idx = jnp.argsort(-r, axis=-1)[:, :C]
        idx_e = jnp.repeat(idx.reshape(B, C, 1), D, axis=2)
        x_sel = jnp.take_along_axis(x, idx_e, axis=1)
        g = _silu(x_sel @ w_gate)
        u = x_sel @ w_up
        y = (g * u) @ w_down
        r_sel = _sigmoid(jnp.take_along_axis(r, idx, axis=1))
        y = y * r_sel.reshape(B, C, 1)
        b_off = (jnp.arange(B) * S).reshape(B, 1)
        flat_idx = (idx + b_off).reshape(B * C)
        zero = (x * 0.0).reshape(B * S, D)
        upd = _scatter_add(zero, flat_idx, y.reshape(B * C, D), axis=0)
        return x + upd.reshape(B, S, D)

    x = A_x
    xn = _layernorm(x, axis=-1)
    s = _A_ref(xn, A_c_kv, A_w_q, A_w_uk, A_w_uv, A_w_o)
    g = _silu(_B_ref(xn, B_w_r, B_w_gate, B_w_up, B_w_down))
    return x + s * g
```

```python
import jax
import jax.numpy as jnp
from jax import lax
import jax.experimental.pallas as pl
import jax.experimental.pallas.tpu as pltpu

_F32 = jnp.float32
_BF16 = jnp.bfloat16
_LANES = 128
_TILE_ROWS = 8
_SLAB = 32
_HG = 16

_WQ, _WUK, _CKV, _WUV, _WG, _WU, _WD, _WO = range(8)

_BLOCK = 8
_BLOCK_START = 6
_BLOCK_STEP = 8
_PARTS = ((1, 0), (3, 1), (1, 0), (3, 1))
_LEAD = 26
_MARGIN = 96
_STEPS = dict(q=(4, 6), uk=(4, 8), qk=(2, 8), pv=(2, 8), uv=(4, 8), up=(4, 8), down=(2, 8), o=(8, 6))
_WO_GROUPS = (18, 7, 4, 2)
_SPLIT_OUT = True
_DEFER = 0
_LAST_PARTS = ((8, ((2, 1),) * 4),)


def _dot(a, b):
    return jnp.dot(a, b, preferred_element_type=_F32)


def _dot_nt(a, b):
    return lax.dot_general(a, b, (((1,), (1,)), ((), ())), preferred_element_type=_F32)


def _iota(shape, axis):
    return lax.broadcasted_iota(jnp.int32, shape, axis)


def _pad_rows(v):
    return jnp.concatenate([v, jnp.zeros((8 - v.shape[0], v.shape[1]), v.dtype)], axis=0)


def _blocks(n_slabs):
    whole = list(range(_BLOCK_START, n_slabs - _BLOCK + 1, _BLOCK))
    ends = [(whole[-1] + _BLOCK, n_slabs), (0, _BLOCK_START)]
    blocks = [[(a, b - a, 1) for a, b in ends if b > a]]
    for i in range(_BLOCK_STEP):
        for start in whole[i::_BLOCK_STEP]:
            blocks.append([])
            for size, priority in _PARTS:
                blocks[-1].append((start, size, priority))
                start += size
    return blocks


class _Stream:
    def __init__(self, order, groups, buf, sems):
        self.groups, self.buf, self.sems = groups, buf, sems
        low = [c for c in order if c[-1]]
        self.todo, low = low[:_LEAD], low[_LEAD:]
        for c in order:
            if not c[-1]:
                self.todo.append(c)
            elif low:
                self.todo.append(low.pop(0))
        self.ready = {g: i + 1 + _MARGIN for i, (g, *_) in enumerate(self.todo)}
        self.done = 0

    def advance(self, count):
        for g, start, to, size, priority in self.todo[self.done:self.done + count]:
            pltpu.make_async_copy(
                self.groups[g][0].at[pl.ds(start, size)],
                self.buf.at[pl.ds(to, size)],
                self.sems.at[g],
            ).start(priority=priority)
        self.done = min(self.done + count, len(self.todo))

    def step(self, stage, i):
        every, count = _STEPS[stage]
        if i % every == every - 1:
            self.advance(count)

    def wait(self, g):
        self.advance(max(self.ready[g] - self.done, 0))
        _, first, size = self.groups[g]
        filled = self.buf.at[pl.ds(first, size)]
        pltpu.make_async_copy(filled, filled, self.sems.at[g]).wait()


def _kernel(
    x_hbm, wr_hbm, wq_hbm, wuk_hbm, ckv_hbm, wuv_hbm, wg_hbm, wu_hbm, wd_hbm, wo_hbm,
    out_hbm,
    buf, expand_v, lhs_v, x_v, wr_v, out_v, ctx_v, head_v, sems, small_sems,
    *, heads, keys, hidden_dim,
):
    B, M = x_v.shape
    D = _LANES
    Dc = wuk_hbm.shape[0]
    n_groups = heads // _HG
    rows = B * _HG
    per_tile = _LANES // _HG
    n_expand = _LANES // per_tile

    sources = [wq_hbm, wuk_hbm, ckv_hbm, wuv_hbm, wg_hbm, wu_hbm, wd_hbm, wo_hbm]
    bases = [0]
    for src in sources:
        bases.append(bases[-1] + src.shape[0])
    q0, uk0, kv0, uv0, g0, u0, d0, o0, _ = bases

    groups = [(src, base, src.shape[0]) for src, base in zip(sources[:_WO], bases)]
    order = [
        (g, start, base + start, size, priority)
        for g, (_, base, n) in enumerate(groups)
        for block in _blocks(n)
        for start, size, priority in block
    ]
    head_slabs = M // _SLAB
    wo_blocks = _blocks(wo_hbm.shape[0])
    wo_blocks.sort(key=lambda block: block[0][0] % head_slabs == 0)
    for k, parts in _LAST_PARTS:
        for block in wo_blocks[-k:]:
            start = block[0][0]
            block.clear()
            for size, priority in parts:
                block.append((start, size, priority))
                start += size
    cuts = [len(wo_blocks) - sum(_WO_GROUPS[i:]) for i in range(len(_WO_GROUPS) + 1)]
    landed = {}
    for g, (a, b) in enumerate(zip([0] + cuts[:-1], cuts), _WO):
        first = o0 + len(landed)
        for start, size, priority in (copy for block in wo_blocks[a:b] for copy in block):
            order.append((g, start, o0 + len(landed), size, priority))
            landed.update({start + i: (g, o0 + len(landed) + i) for i in range(size)})
        groups.append((wo_hbm, first, o0 + len(landed) - first))
    stream = _Stream(order, groups, buf, sems)

    def flat(start, n):
        return buf[start:start + n].reshape(n * _SLAB, _LANES)

    def head_group(base, row0, n, g):
        return buf[base + row0:base + row0 + n, g * _HG:(g + 1) * _HG, :].reshape(n * _HG, D)

    per_slab = _SLAB // _TILE_ROWS

    def cache_tile(k0, n, j):
        first = kv0 + k0 // _TILE_ROWS
        tile = slice(j * _TILE_ROWS, (j + 1) * _TILE_ROWS)
        return buf[first:first + n // _TILE_ROWS, tile, :].reshape(n, _LANES)

    def column_tiles(base):
        per_band = hidden_dim // _LANES // per_slab
        for c in range(per_band):
            slabs = [buf[base + i * per_band + c] for i in range(M // _TILE_ROWS)]
            for r in range(0, _SLAB, _TILE_ROWS):
                yield jnp.concatenate([slab[r:r + _TILE_ROWS] for slab in slabs], axis=0)

    def expand(t):
        return expand_v[t]

    x_cp = pltpu.make_async_copy(x_hbm, x_v, small_sems.at[0])
    wr_cp = pltpu.make_async_copy(wr_hbm, wr_v, small_sems.at[1])
    stream.advance(_LEAD // 2)
    x_cp.start()
    wr_cp.start()
    stream.advance(_MARGIN)

    square = (_LANES, _LANES)
    for t in range(n_expand):
        e = _iota(square, 1) // _HG + t * per_tile == _iota(square, 0)
        expand_v[t] = e.astype(_BF16)
    own_head = _iota((rows, _LANES), 1) % _HG == _iota((rows, _LANES), 0) % _HG

    x_cp.wait()
    wr_cp.wait()
    x = _pad_rows(x_v[...].astype(_F32))
    xc = x - jnp.mean(x, axis=-1, keepdims=True)
    xn_lo = (xc / jnp.sqrt(jnp.mean(xc * xc, axis=-1, keepdims=True) + 1e-5)).astype(_BF16)
    xn = xn_lo.astype(_F32)
    wr = wr_v[...].astype(_F32).reshape(1, M)
    route = jax.nn.sigmoid(jnp.sum(xn * wr, axis=-1, keepdims=True))

    for t in range(M // per_tile):
        m0 = t // n_expand * _LANES
        n = min(_LANES, M - m0)
        rep = _dot(xn_lo[:, m0:m0 + n], expand(t % n_expand)[:n])
        rep = jnp.concatenate(
            [jnp.broadcast_to(rep[b:b + 1], (_HG, _LANES)) for b in range(B)], axis=0
        )
        lhs_v[t] = jnp.where(own_head, rep, 0.0).astype(_BF16)
    stream.wait(_WQ)
    q = [jnp.zeros((rows, D), _F32) for _ in range(n_groups)]
    for t in range(M // per_tile):
        lhs = lhs_v[t]
        for g in range(n_groups):
            q[g] = q[g] + _dot(lhs, head_group(q0, t * per_tile, per_tile, g))
        stream.step("q", t)

    stream.wait(_WUK)
    q_lat = []
    for g in range(n_groups):
        qg = q[g].astype(_BF16)
        tiles = []
        for c0 in range(0, Dc, _LANES):
            acc = jnp.zeros((rows, _LANES), _F32)
            for t in range(n_expand):
                full = _dot_nt(qg, head_group(uk0, c0 + t * per_tile, per_tile, g))
                acc = acc + _dot_nt(jnp.where(own_head, full, 0.0).astype(_BF16), expand(t))
                stream.step("uk", t)
            tiles.append(acc.astype(_BF16))
        q_lat.append(tiles)

    chunk = 256
    lat_tiles = range(Dc // _LANES)

    def scores(b):
        qb = [
            jnp.concatenate([q_lat[g][j][b * _HG:(b + 1) * _HG] for g in range(n_groups)], axis=0)
            for j in lat_tiles
        ]
        chunks = []
        for k0 in range(b * keys, (b + 1) * keys, chunk):
            parts = [_dot_nt(qb[j], cache_tile(k0, chunk, j)) for j in lat_tiles]
            chunks.append(sum(parts[1:], parts[0]))
            stream.step("qk", k0 // chunk)
        return jnp.concatenate(chunks, axis=1) * (D ** -0.5)

    def attend(b, s):
        p = jnp.exp(s - jnp.max(s, axis=-1, keepdims=True))
        denom = jnp.sum(p, axis=-1, keepdims=True)
        p = p.astype(_BF16)
        acc = [jnp.zeros((heads, _LANES), _F32) for _ in lat_tiles]
        for k0 in range(0, keys, chunk):
            acc = [
                a + _dot(p[:, k0:k0 + chunk], cache_tile(b * keys + k0, chunk, j))
                for j, a in enumerate(acc)
            ]
            stream.step("pv", k0 // chunk)
        return [(a / denom).astype(_BF16) for a in acc]

    stream.wait(_CKV)
    lat = []
    s = scores(0)
    for b in range(B):
        ahead = scores(b + 1) if b + 1 < B else None
        lat.append(attend(b, s))
        s = ahead

    stream.wait(_WUV)
    for g in range(n_groups):
        ctx = jnp.zeros((rows, D), _F32)
        for j in range(Dc // _LANES):
            lg = jnp.concatenate([lb[j][g * _HG:(g + 1) * _HG] for lb in lat], axis=0)
            for t in range(n_expand):
                lhs = jnp.where(own_head, _dot(lg, expand(t)), 0.0).astype(_BF16)
                ctx = ctx + _dot(lhs, head_group(uv0, j * _LANES + t * per_tile, per_tile, g))
                stream.step("uv", t)
        ctx_v[:, g * _HG:(g + 1) * _HG, :] = ctx.reshape(B, _HG, D)
    for h in range(heads):
        head_v[h] = _pad_rows(ctx_v[:, h, :]).astype(_BF16)

    def project(base):
        tiles = []
        for j, w in enumerate(column_tiles(base)):
            tiles.append(_dot(xn_lo, w))
            stream.step("up", j)
        return tiles

    stream.wait(_WG)
    gate = [jax.nn.silu(v) for v in project(g0)]
    stream.wait(_WU)
    hidden = [(a * v).astype(_BF16) for a, v in zip(gate, project(u0))]
    stream.wait(_WD)
    y = jnp.zeros(x.shape, _F32)
    for j, w in enumerate(column_tiles(d0)):
        y = y + _dot_nt(hidden[j], w)
        stream.step("down", j)
    mixed = jax.nn.silu(xn + (xn * 0.0 + y * route))

    lane_tiles = [(m0, min(_LANES, M - m0)) for m0 in range(0, M, _LANES)]
    work, done = {}, {}
    for h in range(heads):
        for m0, width in lane_tiles:
            first = h * head_slabs + m0 // _SLAB
            slabs = [landed[slab] for slab in range(first, first + width // _SLAB)]
            g = max(g for g, _ in slabs)
            work.setdefault(g, []).append((h, m0, [to for _, to in slabs]))
            done[m0] = max(done.get(m0, g), g)
    s = {m0: jnp.zeros((x.shape[0], width), _F32) for m0, width in lane_tiles}
    out_cps = []
    pending = []
    for g in range(_WO, len(groups)):
        lhs = {h: head_v[h] for h in sorted({h for h, _, _ in work[g]})}
        stream.wait(g)
        for m0, part in pending:
            s[m0] = s[m0] + part
        pending = []
        late = _DEFER and g < len(groups) - 1 and not [m0 for m0 in done if done[m0] == g]
        for i, (h, m0, slabs) in enumerate(work[g]):
            w = jnp.concatenate([buf[slab] for slab in slabs], axis=0)
            if late and i >= len(work[g]) - _DEFER:
                pending.append((m0, _dot_nt(lhs[h], w)))
            else:
                s[m0] = s[m0] + _dot_nt(lhs[h], w)
            stream.step("o", i)
        final = [(m0, width) for m0, width in lane_tiles if done[m0] == g]
        for m0, width in final:
            cols = slice(m0, m0 + width)
            out_v[:, cols] = (x[:, cols] + s[m0] * mixed[:, cols]).astype(out_v.dtype)[:B]
        if final and _SPLIT_OUT:
            cols = pl.ds(final[0][0], sum(width for _, width in final))
            out_cps.append(pltpu.make_async_copy(
                out_v.at[:, cols], out_hbm.at[:, cols], small_sems.at[len(out_cps)]
            ))
            out_cps[-1].start()
    if not _SPLIT_OUT:
        out_cps.append(pltpu.make_async_copy(out_v, out_hbm, small_sems.at[0]))
        out_cps[-1].start()
    for cp in out_cps:
        cp.wait()


def _slabs(w):
    r, c = w.shape
    w = w.reshape(r // _TILE_ROWS, _TILE_ROWS, c // _LANES, _LANES)
    return w.transpose(0, 2, 1, 3).reshape(-1, _SLAB, _LANES)


@jax.jit
def pallas_recurrent_scan__compressed_kv_cla__moe_arch_mod__decode_kernel(
    A_x: jax.Array,
    A_c_kv: jax.Array,
    A_w_q: jax.Array,
    A_w_uk: jax.Array,
    A_w_uv: jax.Array,
    A_w_o: jax.Array,
    B_x: jax.Array,
    B_w_r: jax.Array,
    B_w_gate: jax.Array,
    B_w_up: jax.Array,
    B_w_down: jax.Array,
):
    del B_x
    B, Sq, M = A_x.shape
    _, Sk, Dc = A_c_kv.shape
    _, H, D = A_w_q.shape
    assert Sq == 1 and H == _SLAB and D == _LANES

    x = A_x.reshape(B, M)
    streamed = [
        A_w_q,
        A_w_uk,
        _slabs(A_c_kv.reshape(B * Sk, Dc)),
        A_w_uv,
        _slabs(B_w_gate),
        _slabs(B_w_up),
        _slabs(B_w_down.T),
        jnp.transpose(A_w_o, (0, 2, 1)).reshape(-1, _SLAB, _LANES),
    ]
    n_slabs = sum(w.shape[0] for w in streamed)

    def kernel(*refs):
        _kernel(*refs, heads=H, keys=Sk, hidden_dim=B_w_gate.shape[1])

    hbm = pl.BlockSpec(memory_space=pltpu.HBM)
    out = pl.pallas_call(
        kernel,
        out_shape=jax.ShapeDtypeStruct((B, M), A_x.dtype),
        in_specs=[hbm] * (2 + len(streamed)),
        out_specs=hbm,
        scratch_shapes=[
            pltpu.VMEM((n_slabs, _SLAB, _LANES), _BF16),
            pltpu.VMEM((_HG, _LANES, _LANES), _BF16),
            pltpu.VMEM((M * _HG // _LANES, B * _HG, _LANES), _BF16),
            pltpu.VMEM(x.shape, x.dtype),
            pltpu.VMEM(B_w_r.shape, B_w_r.dtype),
            pltpu.VMEM(x.shape, x.dtype),
            pltpu.VMEM((B, H, D), _F32),
            pltpu.VMEM((H, 8, D), _BF16),
            pltpu.SemaphoreType.DMA((len(streamed) + len(_WO_GROUPS),)),
            pltpu.SemaphoreType.DMA((3,)),
        ],
        compiler_params=pltpu.CompilerParams(
            vmem_limit_bytes=96 * 1024 * 1024, disable_semaphore_checks=True
        ),
    )(x, B_w_r, *streamed)
    return out.reshape(B, Sq, M)
```

```python
import jax
import jax.numpy as jnp
from jax import lax
import jax.experimental.pallas as pl
import jax.experimental.pallas.tpu as pltpu

_F32 = jnp.float32
_BF16 = jnp.bfloat16
_LANES = 128
_TILE_ROWS = 8
_SLAB = 32
_HG = 16

_WQ, _WUK, _CKV, _WUV, _WG, _WU, _WD, _WO = range(8)

_BLOCK = 8
_BLOCK_START = 6
_BLOCK_STEP = 8
_PARTS = ((2, 0), (6, 1))
_LAST_PARTS = ((2, 1),) * 4
_LAST = 7
_WINDOWS = ((0, .15), (0, .176), (.1, .55), (.3, .62), (.5, .8), (.55, .84), (.6, .907), (.907, 1))
_WO_GROUPS = (18, 8, 4, 3, 2, 2)
_HEAD = 1
_LEAD = 26
_MARGIN = 74
_STEPS = dict(q=(4, 4), uk=(4, 4), qk=(2, 4), pv=(2, 4), uv=(4, 4), up=(4, 4), down=(4, 4), o=(8, 4))


def _dot(a, b):
    return jnp.dot(a, b, preferred_element_type=_F32)


def _dot_nt(a, b):
    return lax.dot_general(a, b, (((1,), (1,)), ((), ())), preferred_element_type=_F32)


def _iota(shape, axis):
    return lax.broadcasted_iota(jnp.int32, shape, axis)


def _pad_rows(v):
    return jnp.concatenate([v, jnp.zeros((8 - v.shape[0], v.shape[1]), v.dtype)], axis=0)


def _cut(start, parts):
    copies = []
    for size, priority in parts:
        copies.append((start, size, priority))
        start += size
    return copies


def _blocks(n_slabs):
    whole = list(range(_BLOCK_START, n_slabs - _BLOCK + 1, _BLOCK))
    blocks = [_cut(start, _PARTS) for i in range(_BLOCK_STEP) for start in whole[i::_BLOCK_STEP]]
    ends = [(whole[-1] + _BLOCK, n_slabs), (0, _BLOCK_START)]
    blocks.insert(len(blocks) // 2, [(a, b - a, 1) for a, b in ends if b > a])
    return blocks


def _moment(operand, i, n):
    first, last = _WINDOWS[operand]
    return first + (last - first) * (i + 0.5) / n


class _Stream:
    def __init__(self, order, groups, buf, sems):
        self.groups, self.buf, self.sems = groups, buf, sems
        head, order = order[:_HEAD], order[_HEAD:]
        low = [c for c in order if c[-1]]
        self.todo, low = head + low[:_LEAD], low[_LEAD:]
        for c in order:
            if not c[-1]:
                self.todo.append(c)
            elif low:
                self.todo.append(low.pop(0))
        self.ready = {g: i + 1 + _MARGIN for i, (g, *_) in enumerate(self.todo)}
        self.done = 0

    def advance(self, count):
        for g, start, to, size, priority in self.todo[self.done:self.done + count]:
            pltpu.make_async_copy(
                self.groups[g][0].at[pl.ds(start, size)],
                self.buf.at[pl.ds(to, size)],
                self.sems.at[g],
            ).start(priority=priority)
        self.done = min(self.done + count, len(self.todo))

    def step(self, stage, i):
        every, count = _STEPS[stage]
        if i % every == every - 1:
            self.advance(count)

    def wait(self, g):
        self.advance(max(self.ready[g] - self.done, 0))
        _, first, size = self.groups[g]
        filled = self.buf.at[pl.ds(first, size)]
        pltpu.make_async_copy(filled, filled, self.sems.at[g]).wait()


def _kernel(
    x_hbm, wr_hbm, wq_hbm, wuk_hbm, ckv_hbm, wuv_hbm, wg_hbm, wu_hbm, wd_hbm, wo_hbm,
    out_hbm,
    buf, expand_v, lhs_v, x_v, wr_v, out_v, ctx_v, head_v, sems, small_sems,
    *, heads, keys, hidden_dim,
):
    B, M = x_v.shape
    D = _LANES
    Dc = wuk_hbm.shape[0]
    n_groups = heads // _HG
    rows = B * _HG
    per_tile = _LANES // _HG
    n_expand = _LANES // per_tile

    sources = [wq_hbm, wuk_hbm, ckv_hbm, wuv_hbm, wg_hbm, wu_hbm, wd_hbm]
    bases = [0]
    for src in sources:
        bases.append(bases[-1] + src.shape[0])
    q0, uk0, kv0, uv0, g0, u0, d0, o0 = bases

    groups = [(src, base, src.shape[0]) for src, base in zip(sources, bases)]
    timed = []
    for g, (_, base, n) in enumerate(groups):
        blocks = _blocks(n)
        for i, block in enumerate(blocks):
            copies = [(g, start, base + start, *rest) for start, *rest in block]
            timed.append((_moment(g, i, len(blocks)), copies))
    head_slabs = M // _SLAB
    blocks = _blocks(wo_hbm.shape[0])
    blocks.sort(key=lambda block: block[0][0] % head_slabs == 0)
    blocks[-_LAST:] = [_cut(block[0][0], _LAST_PARTS) for block in blocks[-_LAST:]]
    cuts = [len(blocks) - sum(_WO_GROUPS[i:]) for i in range(len(_WO_GROUPS) + 1)]
    landed = {}
    for g, (a, b) in enumerate(zip([0] + cuts[:-1], cuts), _WO):
        first = o0 + len(landed)
        for i in range(a, b):
            copies = []
            for start, size, priority in blocks[i]:
                to = o0 + len(landed)
                copies.append((g, start, to, size, priority))
                landed.update({start + j: (g, to + j) for j in range(size)})
            timed.append((_moment(_WO, i, len(blocks)), copies))
        groups.append((wo_hbm, first, o0 + len(landed) - first))
    timed.sort(key=lambda entry: entry[0])
    stream = _Stream([copy for _, copies in timed for copy in copies], groups, buf, sems)

    def head_group(base, row0, n, g):
        return buf[base + row0:base + row0 + n, g * _HG:(g + 1) * _HG, :].reshape(n * _HG, D)

    per_slab = _SLAB // _TILE_ROWS

    def cache_tile(k0, n, j):
        first = kv0 + k0 // _TILE_ROWS
        tile = slice(j * _TILE_ROWS, (j + 1) * _TILE_ROWS)
        return buf[first:first + n // _TILE_ROWS, tile, :].reshape(n, _LANES)

    def column_tile(base, j):
        per_band = hidden_dim // _LANES // per_slab
        tile = slice(j % per_slab * _TILE_ROWS, (j % per_slab + 1) * _TILE_ROWS)
        return jnp.concatenate(
            [buf[base + i * per_band + j // per_slab, tile] for i in range(M // _TILE_ROWS)],
            axis=0,
        )

    x_cp = pltpu.make_async_copy(x_hbm, x_v, small_sems.at[0])
    wr_cp = pltpu.make_async_copy(wr_hbm, wr_v, small_sems.at[1])
    stream.advance(_LEAD // 2)
    x_cp.start()
    wr_cp.start()
    stream.advance(_MARGIN)

    square = (_LANES, _LANES)
    for t in range(n_expand):
        e = _iota(square, 1) // _HG + t * per_tile == _iota(square, 0)
        expand_v[t] = e.astype(_BF16)
    own_head = _iota((rows, _LANES), 1) % _HG == _iota((rows, _LANES), 0) % _HG

    x_cp.wait()
    wr_cp.wait()
    x = _pad_rows(x_v[...].astype(_F32))
    xc = x - jnp.mean(x, axis=-1, keepdims=True)
    xn_lo = (xc / jnp.sqrt(jnp.mean(xc * xc, axis=-1, keepdims=True) + 1e-5)).astype(_BF16)
    xn = xn_lo.astype(_F32)
    wr = wr_v[...].astype(_F32).reshape(1, M)
    route = jax.nn.sigmoid(jnp.sum(xn * wr, axis=-1, keepdims=True))

    for t in range(M // per_tile):
        m0 = t // n_expand * _LANES
        n = min(_LANES, M - m0)
        rep = _dot(xn_lo[:, m0:m0 + n], expand_v[t % n_expand][:n])
        rep = jnp.concatenate(
            [jnp.broadcast_to(rep[b:b + 1], (_HG, _LANES)) for b in range(B)], axis=0
        )
        lhs_v[t] = jnp.where(own_head, rep, 0.0).astype(_BF16)
    stream.wait(_WQ)
    q = [jnp.zeros((rows, D), _F32) for _ in range(n_groups)]
    for t in range(M // per_tile):
        for g in range(n_groups):
            q[g] = q[g] + _dot(lhs_v[t], head_group(q0, t * per_tile, per_tile, g))
        stream.step("q", t)

    stream.wait(_WUK)
    q_lat = []
    for g in range(n_groups):
        qg = q[g].astype(_BF16)
        tiles = []
        for c0 in range(0, Dc, _LANES):
            acc = jnp.zeros((rows, _LANES), _F32)
            for t in range(n_expand):
                full = _dot_nt(qg, head_group(uk0, c0 + t * per_tile, per_tile, g))
                acc = acc + _dot_nt(jnp.where(own_head, full, 0.0).astype(_BF16), expand_v[t])
                stream.step("uk", t)
            tiles.append(acc.astype(_BF16))
        q_lat.append(tiles)

    chunk = 256
    lat_tiles = range(Dc // _LANES)

    def scores(b):
        qb = [
            jnp.concatenate([q_lat[g][j][b * _HG:(b + 1) * _HG] for g in range(n_groups)], axis=0)
            for j in lat_tiles
        ]
        chunks = []
        for k0 in range(0, keys, chunk):
            parts = [_dot_nt(qb[j], cache_tile(b * keys + k0, chunk, j)) for j in lat_tiles]
            chunks.append(sum(parts[1:], parts[0]))
            stream.step("qk", k0 // chunk)
        return jnp.concatenate(chunks, axis=1) * (D ** -0.5)

    def attend(b, s):
        p = jnp.exp(s - jnp.max(s, axis=-1, keepdims=True))
        denom = jnp.sum(p, axis=-1, keepdims=True)
        p = p.astype(_BF16)
        acc = [jnp.zeros((heads, _LANES), _F32) for _ in lat_tiles]
        for k0 in range(0, keys, chunk):
            acc = [
                a + _dot(p[:, k0:k0 + chunk], cache_tile(b * keys + k0, chunk, j))
                for j, a in enumerate(acc)
            ]
            stream.step("pv", k0 // chunk)
        return [(a / denom).astype(_BF16) for a in acc]

    stream.wait(_CKV)
    lat = []
    s = scores(0)
    for b in range(B):
        ahead = scores(b + 1) if b + 1 < B else None
        lat.append(attend(b, s))
        s = ahead

    stream.wait(_WUV)
    for g in range(n_groups):
        ctx = jnp.zeros((rows, D), _F32)
        for j in lat_tiles:
            lg = jnp.concatenate([lb[j][g * _HG:(g + 1) * _HG] for lb in lat], axis=0)
            for t in range(n_expand):
                lhs = jnp.where(own_head, _dot(lg, expand_v[t]), 0.0).astype(_BF16)
                ctx = ctx + _dot(lhs, head_group(uv0, j * _LANES + t * per_tile, per_tile, g))
                stream.step("uv", t)
        ctx_v[:, g * _HG:(g + 1) * _HG, :] = ctx.reshape(B, _HG, D)
    for h in range(heads):
        head_v[h] = _pad_rows(ctx_v[:, h, :]).astype(_BF16)

    hidden_tiles = range(hidden_dim // _LANES)

    def project(base):
        tiles = []
        for j in hidden_tiles:
            tiles.append(_dot(xn_lo, column_tile(base, j)))
            stream.step("up", j)
        return tiles

    stream.wait(_WG)
    gate = [jax.nn.silu(v) for v in project(g0)]
    stream.wait(_WU)
    hidden = [(a * v).astype(_BF16) for a, v in zip(gate, project(u0))]
    stream.wait(_WD)
    y = jnp.zeros(x.shape, _F32)
    for j in hidden_tiles:
        y = y + _dot_nt(hidden[j], column_tile(d0, j))
        stream.step("down", j)
    mixed = jax.nn.silu(xn + (xn * 0.0 + y * route))

    lane_tiles = [(m0, min(_LANES, M - m0)) for m0 in range(0, M, _LANES)]
    work, done = {}, {}
    for h in range(heads):
        for m0, width in lane_tiles:
            first = h * head_slabs + m0 // _SLAB
            slabs = [landed[i] for i in range(first, first + width // _SLAB)]
            g = max(g for g, _ in slabs)
            work.setdefault(g, []).append((h, m0, [to for _, to in slabs]))
            done[m0] = max(done.get(m0, g), g)
    s = {m0: jnp.zeros((x.shape[0], width), _F32) for m0, width in lane_tiles}
    for g in range(_WO, len(groups)):
        lhs = {h: head_v[h] for h in sorted({h for h, _, _ in work[g]})}
        stream.wait(g)
        for i, (h, m0, slabs) in enumerate(work[g]):
            s[m0] = s[m0] + _dot_nt(lhs[h], jnp.concatenate([buf[to] for to in slabs], axis=0))
            stream.step("o", i)
        for m0, width in lane_tiles:
            if done[m0] == g:
                cols = slice(m0, m0 + width)
                out_v[:, cols] = (x[:, cols] + s[m0] * mixed[:, cols]).astype(out_v.dtype)[:B]
    out_cp = pltpu.make_async_copy(out_v, out_hbm, small_sems.at[0])
    out_cp.start()
    out_cp.wait()


def _slabs(w):
    r, c = w.shape
    w = w.reshape(r // _TILE_ROWS, _TILE_ROWS, c // _LANES, _LANES)
    return w.transpose(0, 2, 1, 3).reshape(-1, _SLAB, _LANES)


@jax.jit
def pallas_recurrent_scan__compressed_kv_cla__moe_arch_mod__decode_kernel(
    A_x: jax.Array,
    A_c_kv: jax.Array,
    A_w_q: jax.Array,
    A_w_uk: jax.Array,
    A_w_uv: jax.Array,
    A_w_o: jax.Array,
    B_x: jax.Array,
    B_w_r: jax.Array,
    B_w_gate: jax.Array,
    B_w_up: jax.Array,
    B_w_down: jax.Array,
):
    del B_x
    B, Sq, M = A_x.shape
    _, Sk, Dc = A_c_kv.shape
    _, H, D = A_w_q.shape
    assert Sq == 1 and H == _SLAB and D == _LANES

    x = A_x.reshape(B, M)
    streamed = [
        A_w_q,
        A_w_uk,
        _slabs(A_c_kv.reshape(B * Sk, Dc)),
        A_w_uv,
        _slabs(B_w_gate),
        _slabs(B_w_up),
        _slabs(B_w_down.T),
        jnp.transpose(A_w_o, (0, 2, 1)).reshape(-1, _SLAB, _LANES),
    ]

    def kernel(*refs):
        _kernel(*refs, heads=H, keys=Sk, hidden_dim=B_w_gate.shape[1])

    hbm = pl.BlockSpec(memory_space=pltpu.HBM)
    out = pl.pallas_call(
        kernel,
        out_shape=jax.ShapeDtypeStruct((B, M), A_x.dtype),
        in_specs=[hbm] * (2 + len(streamed)),
        out_specs=hbm,
        scratch_shapes=[
            pltpu.VMEM((sum(w.shape[0] for w in streamed), _SLAB, _LANES), _BF16),
            pltpu.VMEM((_HG, _LANES, _LANES), _BF16),
            pltpu.VMEM((M * _HG // _LANES, B * _HG, _LANES), _BF16),
            pltpu.VMEM(x.shape, x.dtype),
            pltpu.VMEM(B_w_r.shape, B_w_r.dtype),
            pltpu.VMEM(x.shape, x.dtype),
            pltpu.VMEM((B, H, D), _F32),
            pltpu.VMEM((H, 8, D), _BF16),
            pltpu.SemaphoreType.DMA((len(streamed) + len(_WO_GROUPS),)),
            pltpu.SemaphoreType.DMA((2,)),
        ],
        compiler_params=pltpu.CompilerParams(
            vmem_limit_bytes=96 * 1024 * 1024, disable_semaphore_checks=True
        ),
    )(x, B_w_r, *streamed)
    return out.reshape(B, Sq, M)
```

```python
import jax
import jax.numpy as jnp
from jax import lax
import jax.experimental.pallas as pl
import jax.experimental.pallas.tpu as pltpu

_F32 = jnp.float32
_BF16 = jnp.bfloat16
_LANES = 128
_TILE_ROWS = 8
_SLAB = 32
_HG = 16

_WQ, _WUK, _CKV, _WUV, _WG, _WU, _WD, _WO = range(8)

_BLOCK = 8
_BLOCK_START = 6
_BLOCK_STEP = 8
_PARTS = ((2, 0), (6, 1))
_LAST = 7
_LAST_PARTS = ((2, 1),) * 4
_WINDOWS = ((0, .15), (0, .176), (.1, .55), (.3, .62), (.5, .8), (.55, .84), (.6, .907), (.907, 1))
_WO_GROUPS = (18, 8, 4, 4)
_FLAGS = None
_LEAD = 26
_MARGIN = 74
_STEPS = dict(q=(4, 4), uk=(4, 4), qk=(2, 4), pv=(2, 4), uv=(4, 4), up=(4, 4), down=(4, 4), o=(8, 4))


def _dot(a, b):
    return jnp.dot(a, b, preferred_element_type=_F32)


def _dot_nt(a, b):
    return lax.dot_general(a, b, (((1,), (1,)), ((), ())), preferred_element_type=_F32)


def _iota(shape, axis):
    return lax.broadcasted_iota(jnp.int32, shape, axis)


def _pad_rows(v):
    return jnp.concatenate([v, jnp.zeros((8 - v.shape[0], v.shape[1]), v.dtype)], axis=0)


def _cut(start, parts):
    copies = []
    for size, priority in parts:
        copies.append((start, size, priority))
        start += size
    return copies


def _blocks(n_slabs):
    whole = list(range(_BLOCK_START, n_slabs - _BLOCK + 1, _BLOCK))
    blocks = [_cut(start, _PARTS) for i in range(_BLOCK_STEP) for start in whole[i::_BLOCK_STEP]]
    ends = [(whole[-1] + _BLOCK, n_slabs), (0, _BLOCK_START)]
    blocks.insert(len(blocks) // 4, [(a, b - a, 1) for a, b in ends if b > a])
    return blocks


def _moment(operand, i, n):
    first, last = _WINDOWS[operand]
    return first + (last - first) * (i + 0.5) / n


class _Stream:
    def __init__(self, order, groups, buf, sems):
        self.groups, self.buf, self.sems = groups, buf, sems
        low = [c for c in order[1:] if c[-1]]
        self.todo, low = order[:1] + low[:_LEAD], low[_LEAD:]
        for c in order[1:]:
            if not c[-1]:
                self.todo.append(c)
            elif low:
                self.todo.append(low.pop(0))
        self.ready = {g: i + 1 + _MARGIN for i, (g, *_) in enumerate(self.todo)}
        self.done = 0

    def advance(self, count):
        for g, start, to, size, priority in self.todo[self.done:self.done + count]:
            pltpu.make_async_copy(
                self.groups[g][0].at[pl.ds(start, size)],
                self.buf.at[pl.ds(to, size)],
                self.sems.at[g],
            ).start(priority=priority)
        self.done = min(self.done + count, len(self.todo))

    def step(self, stage, i):
        every, count = _STEPS[stage]
        if i % every == every - 1:
            self.advance(count)

    def wait(self, g):
        self.advance(max(self.ready[g] - self.done, 0))
        _, first, size = self.groups[g]
        filled = self.buf.at[pl.ds(first, size)]
        pltpu.make_async_copy(filled, filled, self.sems.at[g]).wait()


def _kernel(
    x_hbm, wr_hbm, wq_hbm, wuk_hbm, ckv_hbm, wuv_hbm, wg_hbm, wu_hbm, wd_hbm, wo_hbm,
    out_hbm,
    buf, expand_v, lhs_v, x_v, wr_v, out_v, ctx_v, head_v, sems, small_sems,
    *, heads, keys, hidden_dim,
):
    B, M = x_v.shape
    D = _LANES
    Dc = wuk_hbm.shape[0]
    n_groups = heads // _HG
    rows = B * _HG
    per_tile = _LANES // _HG
    n_expand = _LANES // per_tile

    sources = [wq_hbm, wuk_hbm, ckv_hbm, wuv_hbm, wg_hbm, wu_hbm, wd_hbm]
    bases = [0]
    for src in sources:
        bases.append(bases[-1] + src.shape[0])
    q0, uk0, kv0, uv0, g0, u0, d0, o0 = bases

    groups = [(src, base, src.shape[0]) for src, base in zip(sources, bases)]
    timed = []
    for g, (_, base, n) in enumerate(groups):
        blocks = _blocks(n)
        for i, block in enumerate(blocks):
            copies = [(g, start, base + start, *rest) for start, *rest in block]
            timed.append((_moment(g, i, len(blocks)), copies))
    head_slabs = M // _SLAB
    blocks = _blocks(wo_hbm.shape[0])
    blocks.sort(key=lambda block: block[0][0] % head_slabs == 0)
    blocks[-_LAST:] = [_cut(block[0][0], _LAST_PARTS) for block in blocks[-_LAST:]]
    cuts = [len(blocks) - sum(_WO_GROUPS[i:]) for i in range(len(_WO_GROUPS) + 1)]
    landed = {}
    for g, (a, b) in enumerate(zip([0] + cuts[:-1], cuts), _WO):
        first = o0 + len(landed)
        for i in range(a, b):
            copies = []
            for start, size, priority in blocks[i]:
                to = o0 + len(landed)
                copies.append((g, start, to, size, priority))
                landed.update({start + j: (g, to + j) for j in range(size)})
            timed.append((_moment(_WO, i, len(blocks)), copies))
        groups.append((wo_hbm, first, o0 + len(landed) - first))
    timed.sort(key=lambda entry: entry[0])
    stream = _Stream([copy for _, copies in timed for copy in copies], groups, buf, sems)

    def head_group(base, row0, n, g):
        return buf[base + row0:base + row0 + n, g * _HG:(g + 1) * _HG, :].reshape(n * _HG, D)

    per_slab = _SLAB // _TILE_ROWS

    def cache_tile(k0, n, j):
        first = kv0 + k0 // _TILE_ROWS
        tile = slice(j * _TILE_ROWS, (j + 1) * _TILE_ROWS)
        return buf[first:first + n // _TILE_ROWS, tile, :].reshape(n, _LANES)

    def column_tile(base, j):
        per_band = hidden_dim // _LANES // per_slab
        tile = slice(j % per_slab * _TILE_ROWS, (j % per_slab + 1) * _TILE_ROWS)
        return jnp.concatenate(
            [buf[base + i * per_band + j // per_slab, tile] for i in range(M // _TILE_ROWS)],
            axis=0,
        )

    x_cp = pltpu.make_async_copy(x_hbm, x_v, small_sems.at[0])
    wr_cp = pltpu.make_async_copy(wr_hbm, wr_v, small_sems.at[1])
    stream.advance(_LEAD // 2)
    x_cp.start()
    wr_cp.start()
    stream.advance(_MARGIN)

    square = (_LANES, _LANES)
    for t in range(n_expand):
        e = _iota(square, 1) // _HG + t * per_tile == _iota(square, 0)
        expand_v[t] = e.astype(_BF16)
    own_head = _iota((rows, _LANES), 1) % _HG == _iota((rows, _LANES), 0) % _HG

    x_cp.wait()
    wr_cp.wait()
    x = _pad_rows(x_v[...].astype(_F32))
    xc = x - jnp.mean(x, axis=-1, keepdims=True)
    xn_lo = (xc / jnp.sqrt(jnp.mean(xc * xc, axis=-1, keepdims=True) + 1e-5)).astype(_BF16)
    xn = xn_lo.astype(_F32)
    wr = wr_v[...].astype(_F32).reshape(1, M)
    route = jax.nn.sigmoid(jnp.sum(xn * wr, axis=-1, keepdims=True))

    for t in range(M // per_tile):
        m0 = t // n_expand * _LANES
        n = min(_LANES, M - m0)
        rep = _dot(xn_lo[:, m0:m0 + n], expand_v[t % n_expand][:n])
        rep = jnp.concatenate(
            [jnp.broadcast_to(rep[b:b + 1], (_HG, _LANES)) for b in range(B)], axis=0
        )
        lhs_v[t] = jnp.where(own_head, rep, 0.0).astype(_BF16)
    stream.wait(_WQ)
    q = [jnp.zeros((rows, D), _F32) for _ in range(n_groups)]
    for t in range(M // per_tile):
        for g in range(n_groups):
            q[g] = q[g] + _dot(lhs_v[t], head_group(q0, t * per_tile, per_tile, g))
        stream.step("q", t)

    stream.wait(_WUK)
    q_lat = []
    for g in range(n_groups):
        qg = q[g].astype(_BF16)
        tiles = []
        for c0 in range(0, Dc, _LANES):
            acc = jnp.zeros((rows, _LANES), _F32)
            for t in range(n_expand):
                full = _dot_nt(qg, head_group(uk0, c0 + t * per_tile, per_tile, g))
                acc = acc + _dot_nt(jnp.where(own_head, full, 0.0).astype(_BF16), expand_v[t])
                stream.step("uk", t)
            tiles.append(acc.astype(_BF16))
        q_lat.append(tiles)

    chunk = 256
    lat_tiles = range(Dc // _LANES)

    def scores(b):
        qb = [
            jnp.concatenate([q_lat[g][j][b * _HG:(b + 1) * _HG] for g in range(n_groups)], axis=0)
            for j in lat_tiles
        ]
        chunks = []
        for k0 in range(0, keys, chunk):
            parts = [_dot_nt(qb[j], cache_tile(b * keys + k0, chunk, j)) for j in lat_tiles]
            chunks.append(sum(parts[1:], parts[0]))
            stream.step("qk", k0 // chunk)
        return jnp.concatenate(chunks, axis=1) * (D ** -0.5)

    def attend(b, s):
        p = jnp.exp(s - jnp.max(s, axis=-1, keepdims=True))
        denom = jnp.sum(p, axis=-1, keepdims=True)
        p = p.astype(_BF16)
        acc = [jnp.zeros((heads, _LANES), _F32) for _ in lat_tiles]
        for k0 in range(0, keys, chunk):
            acc = [
                a + _dot(p[:, k0:k0 + chunk], cache_tile(b * keys + k0, chunk, j))
                for j, a in enumerate(acc)
            ]
            stream.step("pv", k0 // chunk)
        return [(a / denom).astype(_BF16) for a in acc]

    stream.wait(_CKV)
    lat = []
    s = scores(0)
    for b in range(B):
        ahead = scores(b + 1) if b + 1 < B else None
        lat.append(attend(b, s))
        s = ahead

    stream.wait(_WUV)
    for g in range(n_groups):
        ctx = jnp.zeros((rows, D), _F32)
        for j in lat_tiles:
            lg = jnp.concatenate([lb[j][g * _HG:(g + 1) * _HG] for lb in lat], axis=0)
            for t in range(n_expand):
                lhs = jnp.where(own_head, _dot(lg, expand_v[t]), 0.0).astype(_BF16)
                ctx = ctx + _dot(lhs, head_group(uv0, j * _LANES + t * per_tile, per_tile, g))
                stream.step("uv", t)
        ctx_v[:, g * _HG:(g + 1) * _HG, :] = ctx.reshape(B, _HG, D)
    for h in range(heads):
        head_v[h] = _pad_rows(ctx_v[:, h, :]).astype(_BF16)

    hidden_tiles = range(hidden_dim // _LANES)

    def project(base):
        tiles = []
        for j in hidden_tiles:
            tiles.append(_dot(xn_lo, column_tile(base, j)))
            stream.step("up", j)
        return tiles

    stream.wait(_WG)
    gate = [jax.nn.silu(v) for v in project(g0)]
    stream.wait(_WU)
    hidden = [(a * v).astype(_BF16) for a, v in zip(gate, project(u0))]
    stream.wait(_WD)
    y = jnp.zeros(x.shape, _F32)
    for j in hidden_tiles:
        y = y + _dot_nt(hidden[j], column_tile(d0, j))
        stream.step("down", j)
    mixed = jax.nn.silu(xn + (xn * 0.0 + y * route))

    lane_tiles = [(m0, min(_LANES, M - m0)) for m0 in range(0, M, _LANES)]
    work, done = {}, {}
    for h in range(heads):
        for m0, width in lane_tiles:
            first = h * head_slabs + m0 // _SLAB
            slabs = [landed[i] for i in range(first, first + width // _SLAB)]
            g = max(g for g, _ in slabs)
            work.setdefault(g, []).append((h, m0, [to for _, to in slabs]))
            done[m0] = max(done.get(m0, g), g)
    s = {m0: jnp.zeros((x.shape[0], width), _F32) for m0, width in lane_tiles}
    last = len(groups) - 1
    late = min(m0 for m0 in done if done[m0] < last)
    out_cps = [
        pltpu.make_async_copy(out_v.at[:, cols], out_hbm.at[:, cols], small_sems.at[i])
        for i, cols in enumerate([pl.ds(late, M - late), pl.ds(0, late)])
    ]
    for g in range(_WO, len(groups)):
        lhs = {h: head_v[h] for h in sorted({h for h, _, _ in work[g]})}
        stream.wait(g)
        if g == last:
            out_cps[0].start()
        for i, (h, m0, slabs) in enumerate(work[g]):
            s[m0] = s[m0] + _dot_nt(lhs[h], jnp.concatenate([buf[to] for to in slabs], axis=0))
            stream.step("o", i)
        for m0, width in lane_tiles:
            if done[m0] == g:
                cols = slice(m0, m0 + width)
                out_v[:, cols] = (x[:, cols] + s[m0] * mixed[:, cols]).astype(out_v.dtype)[:B]
    out_cps[1].start()
    for cp in out_cps:
        cp.wait()


def _slabs(w):
    r, c = w.shape
    w = w.reshape(r // _TILE_ROWS, _TILE_ROWS, c // _LANES, _LANES)
    return w.transpose(0, 2, 1, 3).reshape(-1, _SLAB, _LANES)


@jax.jit
def pallas_recurrent_scan__compressed_kv_cla__moe_arch_mod__decode_kernel(
    A_x: jax.Array,
    A_c_kv: jax.Array,
    A_w_q: jax.Array,
    A_w_uk: jax.Array,
    A_w_uv: jax.Array,
    A_w_o: jax.Array,
    B_x: jax.Array,
    B_w_r: jax.Array,
    B_w_gate: jax.Array,
    B_w_up: jax.Array,
    B_w_down: jax.Array,
):
    del B_x
    B, Sq, M = A_x.shape
    _, Sk, Dc = A_c_kv.shape
    _, H, D = A_w_q.shape
    assert Sq == 1 and H == _SLAB and D == _LANES

    x = A_x.reshape(B, M)
    streamed = [
        A_w_q,
        A_w_uk,
        _slabs(A_c_kv.reshape(B * Sk, Dc)),
        A_w_uv,
        _slabs(B_w_gate),
        _slabs(B_w_up),
        _slabs(B_w_down.T),
        jnp.transpose(A_w_o, (0, 2, 1)).reshape(-1, _SLAB, _LANES),
    ]

    def kernel(*refs):
        _kernel(*refs, heads=H, keys=Sk, hidden_dim=B_w_gate.shape[1])

    hbm = pl.BlockSpec(memory_space=pltpu.HBM)
    out = pl.pallas_call(
        kernel,
        out_shape=jax.ShapeDtypeStruct((B, M), A_x.dtype),
        in_specs=[hbm] * (2 + len(streamed)),
        out_specs=hbm,
        scratch_shapes=[
            pltpu.VMEM((sum(w.shape[0] for w in streamed), _SLAB, _LANES), _BF16),
            pltpu.VMEM((_HG, _LANES, _LANES), _BF16),
            pltpu.VMEM((M * _HG // _LANES, B * _HG, _LANES), _BF16),
            pltpu.VMEM(x.shape, x.dtype),
            pltpu.VMEM(B_w_r.shape, B_w_r.dtype),
            pltpu.VMEM(x.shape, x.dtype),
            pltpu.VMEM((B, H, D), _F32),
            pltpu.VMEM((H, 8, D), _BF16),
            pltpu.SemaphoreType.DMA((len(streamed) + len(_WO_GROUPS),)),
            pltpu.SemaphoreType.DMA((2,)),
        ],
        compiler_params=pltpu.CompilerParams(
            vmem_limit_bytes=96 * 1024 * 1024, disable_semaphore_checks=True, flags=_FLAGS
        ),
    )(x, B_w_r, *streamed)
    return out.reshape(B, Sq, M)
```

```python
import jax
import jax.numpy as jnp
from jax import lax
import jax.experimental.pallas as pl
import jax.experimental.pallas.tpu as pltpu

_F32 = jnp.float32
_BF16 = jnp.bfloat16
_LANES = 128
_TILE_ROWS = 8
_SLAB = 32
_HG = 16

_WQ, _WUK, _CKV, _WUV, _WG, _WU, _WD, _WO = range(8)

_BLOCK = 8
_BLOCK_START = 6
_BLOCK_STEP = 8
_PARTS = ((2, 0), (6, 1))
_LAST = 7
_LAST_PARTS = ((2, 1),) * 4
_WINDOWS = ((0, .15), (0, .176), (.1, .55), (.3, .62), (.5, .8), (.55, .84), (.6, .907), (.907, 1))
_WO_GROUPS = (18, 8, 4, 4)
_FLAGS = None
_LEAD = 26
_MARGIN = 74
_STEPS = dict(q=(4, 4), uk=(4, 4), qk=(2, 4), pv=(2, 4), uv=(4, 4), up=(4, 4), down=(4, 4), o=(8, 4))


def _dot(a, b):
    return jnp.dot(a, b, preferred_element_type=_F32)


def _dot_nt(a, b):
    return lax.dot_general(a, b, (((1,), (1,)), ((), ())), preferred_element_type=_F32)


def _iota(shape, axis):
    return lax.broadcasted_iota(jnp.int32, shape, axis)


def _pad_rows(v):
    return jnp.concatenate([v, jnp.zeros((8 - v.shape[0], v.shape[1]), v.dtype)], axis=0)


def _cut(start, parts):
    copies = []
    for size, priority in parts:
        copies.append((start, size, priority))
        start += size
    return copies


def _blocks(n_slabs):
    whole = list(range(_BLOCK_START, n_slabs - _BLOCK + 1, _BLOCK))
    blocks = [_cut(start, _PARTS) for i in range(_BLOCK_STEP) for start in whole[i::_BLOCK_STEP]]
    ends = [(whole[-1] + _BLOCK, n_slabs), (0, _BLOCK_START)]
    blocks.insert(len(blocks) // 4, [(a, b - a, 1) for a, b in ends if b > a])
    return blocks


def _moment(operand, i, n):
    first, last = _WINDOWS[operand]
    return first + (last - first) * (i + 0.5) / n


class _Stream:
    def __init__(self, order, groups, buf, sems):
        self.groups, self.buf, self.sems = groups, buf, sems
        low = [c for c in order[1:] if c[-1]]
        self.todo, low = order[:1] + low[:_LEAD], low[_LEAD:]
        for c in order[1:]:
            if not c[-1]:
                self.todo.append(c)
            elif low:
                self.todo.append(low.pop(0))
        self.ready = {g: i + 1 + _MARGIN for i, (g, *_) in enumerate(self.todo)}
        self.done = 0

    def advance(self, count):
        for g, start, to, size, priority in self.todo[self.done:self.done + count]:
            pltpu.make_async_copy(
                self.groups[g][0].at[pl.ds(start, size)],
                self.buf.at[pl.ds(to, size)],
                self.sems.at[g],
            ).start(priority=priority)
        self.done = min(self.done + count, len(self.todo))

    def step(self, stage, i):
        every, count = _STEPS[stage]
        if i % every == every - 1:
            self.advance(count)

    def wait(self, g):
        self.advance(max(self.ready[g] - self.done, 0))
        _, first, size = self.groups[g]
        filled = self.buf.at[pl.ds(first, size)]
        pltpu.make_async_copy(filled, filled, self.sems.at[g]).wait()


def _kernel(
    x_hbm, wr_hbm, wq_hbm, wuk_hbm, ckv_hbm, wuv_hbm, wg_hbm, wu_hbm, wd_hbm, wo_hbm,
    out_hbm,
    buf, expand_v, lhs_v, x_v, wr_v, out_v, ctx_v, head_v, sems, small_sems,
    *, heads, keys, hidden_dim,
):
    B, M = x_v.shape
    D = _LANES
    Dc = wuk_hbm.shape[0]
    n_groups = heads // _HG
    rows = B * _HG
    per_tile = _LANES // _HG
    n_expand = _LANES // per_tile

    sources = [wq_hbm, wuk_hbm, ckv_hbm, wuv_hbm, wg_hbm, wu_hbm, wd_hbm]
    bases = [0]
    for src in sources:
        bases.append(bases[-1] + src.shape[0])
    q0, uk0, kv0, uv0, g0, u0, d0, o0 = bases

    groups = [(src, base, src.shape[0]) for src, base in zip(sources, bases)]
    timed = []
    for g, (_, base, n) in enumerate(groups):
        blocks = _blocks(n)
        for i, block in enumerate(blocks):
            copies = [(g, start, base + start, *rest) for start, *rest in block]
            timed.append((_moment(g, i, len(blocks)), copies))
    head_slabs = M // _SLAB
    blocks = _blocks(wo_hbm.shape[0])
    blocks.sort(key=lambda block: block[0][0] % head_slabs == 0)
    blocks[-_LAST:] = [_cut(block[0][0], _LAST_PARTS) for block in blocks[-_LAST:]]
    cuts = [len(blocks) - sum(_WO_GROUPS[i:]) for i in range(len(_WO_GROUPS) + 1)]
    landed = {}
    for g, (a, b) in enumerate(zip([0] + cuts[:-1], cuts), _WO):
        first = o0 + len(landed)
        for i in range(a, b):
            copies = []
            for start, size, priority in blocks[i]:
                to = o0 + len(landed)
                copies.append((g, start, to, size, priority))
                landed.update({start + j: (g, to + j) for j in range(size)})
            timed.append((_moment(_WO, i, len(blocks)), copies))
        groups.append((wo_hbm, first, o0 + len(landed) - first))
    timed.sort(key=lambda entry: entry[0])
    stream = _Stream([copy for _, copies in timed for copy in copies], groups, buf, sems)

    def head_group(base, row0, n, g):
        return buf[base + row0:base + row0 + n, g * _HG:(g + 1) * _HG, :].reshape(n * _HG, D)

    per_slab = _SLAB // _TILE_ROWS

    def cache_tile(k0, n, j):
        first = kv0 + k0 // _TILE_ROWS
        tile = slice(j * _TILE_ROWS, (j + 1) * _TILE_ROWS)
        return buf[first:first + n // _TILE_ROWS, tile, :].reshape(n, _LANES)

    def column_tile(base, j):
        per_band = hidden_dim // _LANES // per_slab
        tile = slice(j % per_slab * _TILE_ROWS, (j % per_slab + 1) * _TILE_ROWS)
        return jnp.concatenate(
            [buf[base + i * per_band + j // per_slab, tile] for i in range(M // _TILE_ROWS)],
            axis=0,
        )

    x_cp = pltpu.make_async_copy(x_hbm, x_v, small_sems.at[0])
    wr_cp = pltpu.make_async_copy(wr_hbm, wr_v, small_sems.at[1])
    stream.advance(_LEAD // 2)
    x_cp.start()
    wr_cp.start()
    stream.advance(_MARGIN)

    square = (_LANES, _LANES)
    for t in range(n_expand):
        e = _iota(square, 1) // _HG + t * per_tile == _iota(square, 0)
        expand_v[t] = e.astype(_BF16)
    own_head = _iota((rows, _LANES), 1) % _HG == _iota((rows, _LANES), 0) % _HG

    x_cp.wait()
    wr_cp.wait()
    x = _pad_rows(x_v[...].astype(_F32))
    xc = x - jnp.mean(x, axis=-1, keepdims=True)
    xn_lo = (xc / jnp.sqrt(jnp.mean(xc * xc, axis=-1, keepdims=True) + 1e-5)).astype(_BF16)
    xn = xn_lo.astype(_F32)
    wr = wr_v[...].astype(_F32).reshape(1, M)
    route = jax.nn.sigmoid(jnp.sum(xn * wr, axis=-1, keepdims=True))

    for t in range(M // per_tile):
        m0 = t // n_expand * _LANES
        n = min(_LANES, M - m0)
        rep = _dot(xn_lo[:, m0:m0 + n], expand_v[t % n_expand][:n])
        rep = jnp.concatenate(
            [jnp.broadcast_to(rep[b:b + 1], (_HG, _LANES)) for b in range(B)], axis=0
        )
        lhs_v[t] = jnp.where(own_head, rep, 0.0).astype(_BF16)
    stream.wait(_WQ)
    q = [jnp.zeros((rows, D), _F32) for _ in range(n_groups)]
    for t in range(M // per_tile):
        for g in range(n_groups):
            q[g] = q[g] + _dot(lhs_v[t], head_group(q0, t * per_tile, per_tile, g))
        stream.step("q", t)

    stream.wait(_WUK)
    q_lat = []
    for g in range(n_groups):
        qg = q[g].astype(_BF16)
        tiles = []
        for c0 in range(0, Dc, _LANES):
            acc = jnp.zeros((rows, _LANES), _F32)
            for t in range(n_expand):
                full = _dot_nt(qg, head_group(uk0, c0 + t * per_tile, per_tile, g))
                acc = acc + _dot_nt(jnp.where(own_head, full, 0.0).astype(_BF16), expand_v[t])
                stream.step("uk", t)
            tiles.append(acc.astype(_BF16))
        q_lat.append(tiles)

    chunk = 256
    lat_tiles = range(Dc // _LANES)

    def scores(b):
        qb = [
            jnp.concatenate([q_lat[g][j][b * _HG:(b + 1) * _HG] for g in range(n_groups)], axis=0)
            for j in lat_tiles
        ]
        chunks = []
        for k0 in range(0, keys, chunk):
            parts = [_dot_nt(qb[j], cache_tile(b * keys + k0, chunk, j)) for j in lat_tiles]
            chunks.append(sum(parts[1:], parts[0]))
            stream.step("qk", k0 // chunk)
        return jnp.concatenate(chunks, axis=1) * (D ** -0.5)

    def attend(b, s):
        p = jnp.exp(s - jnp.max(s, axis=-1, keepdims=True))
        denom = jnp.sum(p, axis=-1, keepdims=True)
        p = p.astype(_BF16)
        acc = [jnp.zeros((heads, _LANES), _F32) for _ in lat_tiles]
        for k0 in range(0, keys, chunk):
            acc = [
                a + _dot(p[:, k0:k0 + chunk], cache_tile(b * keys + k0, chunk, j))
                for j, a in enumerate(acc)
            ]
            stream.step("pv", k0 // chunk)
        return [(a / denom).astype(_BF16) for a in acc]

    stream.wait(_CKV)
    lat = []
    s = scores(0)
    for b in range(B):
        ahead = scores(b + 1) if b + 1 < B else None
        lat.append(attend(b, s))
        s = ahead

    stream.wait(_WUV)
    for g in range(n_groups):
        ctx = jnp.zeros((rows, D), _F32)
        for j in lat_tiles:
            lg = jnp.concatenate([lb[j][g * _HG:(g + 1) * _HG] for lb in lat], axis=0)
            for t in range(n_expand):
                lhs = jnp.where(own_head, _dot(lg, expand_v[t]), 0.0).astype(_BF16)
                ctx = ctx + _dot(lhs, head_group(uv0, j * _LANES + t * per_tile, per_tile, g))
                stream.step("uv", t)
        ctx_v[:, g * _HG:(g + 1) * _HG, :] = ctx.reshape(B, _HG, D)
    for h in range(heads):
        head_v[h] = _pad_rows(ctx_v[:, h, :]).astype(_BF16)

    hidden_tiles = range(hidden_dim // _LANES)

    def project(base):
        tiles = []
        for j in hidden_tiles:
            tiles.append(_dot(xn_lo, column_tile(base, j)))
            stream.step("up", j)
        return tiles

    stream.wait(_WG)
    gate = [jax.nn.silu(v) for v in project(g0)]
    stream.wait(_WU)
    hidden = [(a * v).astype(_BF16) for a, v in zip(gate, project(u0))]
    stream.wait(_WD)
    y = jnp.zeros(x.shape, _F32)
    for j in hidden_tiles:
        y = y + _dot_nt(hidden[j], column_tile(d0, j))
        stream.step("down", j)
    mixed = jax.nn.silu(xn + (xn * 0.0 + y * route))

    lane_tiles = [(m0, min(_LANES, M - m0)) for m0 in range(0, M, _LANES)]
    work, done = {}, {}
    for h in range(heads):
        for m0, width in lane_tiles:
            first = h * head_slabs + m0 // _SLAB
            slabs = [landed[i] for i in range(first, first + width // _SLAB)]
            g = max(g for g, _ in slabs)
            work.setdefault(g, []).append((h, m0, [to for _, to in slabs]))
            done[m0] = max(done.get(m0, g), g)
    s = {m0: jnp.zeros((x.shape[0], width), _F32) for m0, width in lane_tiles}
    for g in range(_WO, len(groups)):
        lhs = {h: head_v[h] for h in sorted({h for h, _, _ in work[g]})}
        stream.wait(g)
        for i, (h, m0, slabs) in enumerate(work[g]):
            s[m0] = s[m0] + _dot_nt(lhs[h], jnp.concatenate([buf[to] for to in slabs], axis=0))
            stream.step("o", i)
        for m0, width in lane_tiles:
            if done[m0] == g:
                cols = slice(m0, m0 + width)
                out_v[:, cols] = (x[:, cols] + s[m0] * mixed[:, cols]).astype(out_v.dtype)[:B]
    out_cp = pltpu.make_async_copy(out_v, out_hbm, small_sems.at[0])
    out_cp.start()
    out_cp.wait()


def _slabs(w):
    r, c = w.shape
    w = w.reshape(r // _TILE_ROWS, _TILE_ROWS, c // _LANES, _LANES)
    return w.transpose(0, 2, 1, 3).reshape(-1, _SLAB, _LANES)


@jax.jit
def pallas_recurrent_scan__compressed_kv_cla__moe_arch_mod__decode_kernel(
    A_x: jax.Array,
    A_c_kv: jax.Array,
    A_w_q: jax.Array,
    A_w_uk: jax.Array,
    A_w_uv: jax.Array,
    A_w_o: jax.Array,
    B_x: jax.Array,
    B_w_r: jax.Array,
    B_w_gate: jax.Array,
    B_w_up: jax.Array,
    B_w_down: jax.Array,
):
    del B_x
    B, Sq, M = A_x.shape
    _, Sk, Dc = A_c_kv.shape
    _, H, D = A_w_q.shape
    assert Sq == 1 and H == _SLAB and D == _LANES

    x = A_x.reshape(B, M)
    streamed = [
        A_w_q,
        A_w_uk,
        _slabs(A_c_kv.reshape(B * Sk, Dc)),
        A_w_uv,
        _slabs(B_w_gate),
        _slabs(B_w_up),
        _slabs(B_w_down.T),
        jnp.transpose(A_w_o, (0, 2, 1)).reshape(-1, _SLAB, _LANES),
    ]

    def kernel(*refs):
        _kernel(*refs, heads=H, keys=Sk, hidden_dim=B_w_gate.shape[1])

    hbm = pl.BlockSpec(memory_space=pltpu.HBM)
    out = pl.pallas_call(
        kernel,
        out_shape=jax.ShapeDtypeStruct((B, M), A_x.dtype),
        in_specs=[hbm] * (2 + len(streamed)),
        out_specs=hbm,
        scratch_shapes=[
            pltpu.VMEM((sum(w.shape[0] for w in streamed), _SLAB, _LANES), _BF16),
            pltpu.VMEM((_HG, _LANES, _LANES), _BF16),
            pltpu.VMEM((M * _HG // _LANES, B * _HG, _LANES), _BF16),
            pltpu.VMEM(x.shape, x.dtype),
            pltpu.VMEM(B_w_r.shape, B_w_r.dtype),
            pltpu.VMEM(x.shape, x.dtype),
            pltpu.VMEM((B, H, D), _F32),
            pltpu.VMEM((H, 8, D), _BF16),
            pltpu.SemaphoreType.DMA((len(streamed) + len(_WO_GROUPS),)),
            pltpu.SemaphoreType.DMA((2,)),
        ],
        compiler_params=pltpu.CompilerParams(
            vmem_limit_bytes=96 * 1024 * 1024, disable_semaphore_checks=True, flags=_FLAGS
        ),
    )(x, B_w_r, *streamed)
    return out.reshape(B, Sq, M)
```

```python
import jax
import jax.numpy as jnp
from jax import lax
import jax.experimental.pallas as pl
import jax.experimental.pallas.tpu as pltpu

_F32 = jnp.float32
_BF16 = jnp.bfloat16
_LANES = 128
_TILE_ROWS = 8
_SLAB = 32
_HG = 16

_WQ, _WUK, _CKV, _WUV, _WG, _WU, _WD, _WO = range(8)

_BLOCK = 8
_BLOCK_START = 6
_BLOCK_STEP = 8
_PARTS = ((2, 0), (6, 1))
_LAST = 6
_LAST_PARTS = ((2, 1), (1, 1), (2, 1), (1, 1), (2, 1))
_WINDOWS = ((0, .15), (0, .176), (.1, .55), (.3, .62), (.5, .8), (.55, .84), (.6, .907), (.907, 1))
_WO_GROUPS = (18, 8, 4, 4)
_LEAD = 26
_MARGIN = 74
_STEPS = dict(
    q=(4, 4), uk=(4, 4), qk=(2, 4), pv=(2, 4), uv=(4, 4), up=(4, 4), down=(4, 4), o=(8, 4)
)


def _dot(a, b):
    return jnp.dot(a, b, preferred_element_type=_F32)


def _dot_nt(a, b):
    return lax.dot_general(a, b, (((1,), (1,)), ((), ())), preferred_element_type=_F32)


def _iota(shape, axis):
    return lax.broadcasted_iota(jnp.int32, shape, axis)


def _pad_rows(v):
    return jnp.concatenate([v, jnp.zeros((8 - v.shape[0], v.shape[1]), v.dtype)], axis=0)


def _cut(start, parts):
    copies = []
    for size, priority in parts:
        copies.append((start, size, priority))
        start += size
    return copies


def _blocks(n_slabs):
    whole = list(range(_BLOCK_START, n_slabs - _BLOCK + 1, _BLOCK))
    blocks = [_cut(start, _PARTS) for i in range(_BLOCK_STEP) for start in whole[i::_BLOCK_STEP]]
    ends = [(whole[-1] + _BLOCK, n_slabs), (0, _BLOCK_START)]
    blocks.insert(len(blocks) // 4, [(a, b - a, 1) for a, b in ends if b > a])
    return blocks


def _moment(operand, i, n):
    first, last = _WINDOWS[operand]
    return first + (last - first) * (i + 0.5) / n


class _Stream:
    def __init__(self, order, groups, buf, sems):
        self.groups, self.buf, self.sems = groups, buf, sems
        low = [c for c in order[1:] if c[-1]]
        self.todo, low = order[:1] + low[:_LEAD], low[_LEAD:]
        for c in order[1:]:
            if not c[-1]:
                self.todo.append(c)
            elif low:
                self.todo.append(low.pop(0))
        self.ready = {g: i + 1 + _MARGIN for i, (g, *_) in enumerate(self.todo)}
        self.done = 0

    def advance(self, count):
        for g, start, to, size, priority in self.todo[self.done:self.done + count]:
            pltpu.make_async_copy(
                self.groups[g][0].at[pl.ds(start, size)],
                self.buf.at[pl.ds(to, size)],
                self.sems.at[g],
            ).start(priority=priority)
        self.done = min(self.done + count, len(self.todo))

    def step(self, stage, i):
        every, count = _STEPS[stage]
        if i % every == every - 1:
            self.advance(count)

    def wait(self, g):
        self.advance(max(self.ready[g] - self.done, 0))
        _, first, size = self.groups[g]
        filled = self.buf.at[pl.ds(first, size)]
        pltpu.make_async_copy(filled, filled, self.sems.at[g]).wait()


def _kernel(
    x_hbm, wr_hbm, wq_hbm, wuk_hbm, ckv_hbm, wuv_hbm, wg_hbm, wu_hbm, wd_hbm, wo_hbm,
    out_hbm,
    buf, expand_v, lhs_v, x_v, wr_v, out_v, ctx_v, head_v, sems, small_sems,
    *, heads, keys, hidden_dim,
):
    B, M = x_v.shape
    D = _LANES
    Dc = wuk_hbm.shape[0]
    n_groups = heads // _HG
    rows = B * _HG
    per_tile = _LANES // _HG
    n_expand = _LANES // per_tile

    sources = [wq_hbm, wuk_hbm, ckv_hbm, wuv_hbm, wg_hbm, wu_hbm, wd_hbm]
    bases = [0]
    for src in sources:
        bases.append(bases[-1] + src.shape[0])
    q0, uk0, kv0, uv0, g0, u0, d0, o0 = bases

    groups = [(src, base, src.shape[0]) for src, base in zip(sources, bases)]
    timed = []
    for g, (_, base, n) in enumerate(groups):
        blocks = _blocks(n)
        for i, block in enumerate(blocks):
            copies = [(g, start, base + start, *rest) for start, *rest in block]
            timed.append((_moment(g, i, len(blocks)), copies))
    head_slabs = M // _SLAB
    blocks = _blocks(wo_hbm.shape[0])
    blocks.sort(key=lambda block: block[0][0] % head_slabs == 0)
    blocks[-_LAST:] = [_cut(block[0][0], _LAST_PARTS) for block in blocks[-_LAST:]]
    cuts = [len(blocks) - sum(_WO_GROUPS[i:]) for i in range(len(_WO_GROUPS) + 1)]
    landed = {}
    for g, (a, b) in enumerate(zip([0] + cuts[:-1], cuts), _WO):
        first = o0 + len(landed)
        for i in range(a, b):
            copies = []
            for start, size, priority in blocks[i]:
                to = o0 + len(landed)
                copies.append((g, start, to, size, priority))
                landed.update({start + j: (g, to + j) for j in range(size)})
            timed.append((_moment(_WO, i, len(blocks)), copies))
        groups.append((wo_hbm, first, o0 + len(landed) - first))
    timed.sort(key=lambda entry: entry[0])
    stream = _Stream([copy for _, copies in timed for copy in copies], groups, buf, sems)

    def head_group(base, row0, n, g):
        return buf[base + row0:base + row0 + n, g * _HG:(g + 1) * _HG, :].reshape(n * _HG, D)

    per_slab = _SLAB // _TILE_ROWS

    def cache_tile(k0, n, j):
        first = kv0 + k0 // _TILE_ROWS
        tile = slice(j * _TILE_ROWS, (j + 1) * _TILE_ROWS)
        return buf[first:first + n // _TILE_ROWS, tile, :].reshape(n, _LANES)

    def column_tile(base, j):
        per_band = hidden_dim // _LANES // per_slab
        tile = slice(j % per_slab * _TILE_ROWS, (j % per_slab + 1) * _TILE_ROWS)
        return jnp.concatenate(
            [buf[base + i * per_band + j // per_slab, tile] for i in range(M // _TILE_ROWS)],
            axis=0,
        )

    x_cp = pltpu.make_async_copy(x_hbm, x_v, small_sems.at[0])
    wr_cp = pltpu.make_async_copy(wr_hbm, wr_v, small_sems.at[1])
    stream.advance(_LEAD // 2)
    x_cp.start()
    wr_cp.start()
    stream.advance(_MARGIN)

    square = (_LANES, _LANES)
    for t in range(n_expand):
        e = _iota(square, 1) // _HG + t * per_tile == _iota(square, 0)
        expand_v[t] = e.astype(_BF16)
    own_head = _iota((rows, _LANES), 1) % _HG == _iota((rows, _LANES), 0) % _HG

    x_cp.wait()
    wr_cp.wait()
    x = _pad_rows(x_v[...].astype(_F32))
    xc = x - jnp.mean(x, axis=-1, keepdims=True)
    xn_lo = (xc / jnp.sqrt(jnp.mean(xc * xc, axis=-1, keepdims=True) + 1e-5)).astype(_BF16)
    xn = xn_lo.astype(_F32)
    wr = wr_v[...].astype(_F32).reshape(1, M)
    route = jax.nn.sigmoid(jnp.sum(xn * wr, axis=-1, keepdims=True))

    for t in range(M // per_tile):
        m0 = t // n_expand * _LANES
        n = min(_LANES, M - m0)
        rep = _dot(xn_lo[:, m0:m0 + n], expand_v[t % n_expand][:n])
        rep = jnp.concatenate(
            [jnp.broadcast_to(rep[b:b + 1], (_HG, _LANES)) for b in range(B)], axis=0
        )
        lhs_v[t] = jnp.where(own_head, rep, 0.0).astype(_BF16)
    stream.wait(_WQ)
    q = [jnp.zeros((rows, D), _F32) for _ in range(n_groups)]
    for t in range(M // per_tile):
        for g in range(n_groups):
            q[g] = q[g] + _dot(lhs_v[t], head_group(q0, t * per_tile, per_tile, g))
        stream.step("q", t)

    stream.wait(_WUK)
    q_lat = []
    for g in range(n_groups):
        qg = q[g].astype(_BF16)
        tiles = []
        for c0 in range(0, Dc, _LANES):
            acc = jnp.zeros((rows, _LANES), _F32)
            for t in range(n_expand):
                full = _dot_nt(qg, head_group(uk0, c0 + t * per_tile, per_tile, g))
                acc = acc + _dot_nt(jnp.where(own_head, full, 0.0).astype(_BF16), expand_v[t])
                stream.step("uk", t)
            tiles.append(acc.astype(_BF16))
        q_lat.append(tiles)

    chunk = 256
    lat_tiles = range(Dc // _LANES)

    def scores(b):
        qb = [
            jnp.concatenate([q_lat[g][j][b * _HG:(b + 1) * _HG] for g in range(n_groups)], axis=0)
            for j in lat_tiles
        ]
        chunks = []
        for k0 in range(0, keys, chunk):
            parts = [_dot_nt(qb[j], cache_tile(b * keys + k0, chunk, j)) for j in lat_tiles]
            chunks.append(sum(parts[1:], parts[0]))
            stream.step("qk", k0 // chunk)
        return jnp.concatenate(chunks, axis=1) * (D ** -0.5)

    def attend(b, s):
        p = jnp.exp(s - jnp.max(s, axis=-1, keepdims=True))
        denom = jnp.sum(p, axis=-1, keepdims=True)
        p = p.astype(_BF16)
        acc = [jnp.zeros((heads, _LANES), _F32) for _ in lat_tiles]
        for k0 in range(0, keys, chunk):
            acc = [
                a + _dot(p[:, k0:k0 + chunk], cache_tile(b * keys + k0, chunk, j))
                for j, a in enumerate(acc)
            ]
            stream.step("pv", k0 // chunk)
        return [(a / denom).astype(_BF16) for a in acc]

    stream.wait(_CKV)
    lat = []
    s = scores(0)
    for b in range(B):
        ahead = scores(b + 1) if b + 1 < B else None
        lat.append(attend(b, s))
        s = ahead

    stream.wait(_WUV)
    for g in range(n_groups):
        ctx = jnp.zeros((rows, D), _F32)
        for j in lat_tiles:
            lg = jnp.concatenate([lb[j][g * _HG:(g + 1) * _HG] for lb in lat], axis=0)
            for t in range(n_expand):
                lhs = jnp.where(own_head, _dot(lg, expand_v[t]), 0.0).astype(_BF16)
                ctx = ctx + _dot(lhs, head_group(uv0, j * _LANES + t * per_tile, per_tile, g))
                stream.step("uv", t)
        ctx_v[:, g * _HG:(g + 1) * _HG, :] = ctx.reshape(B, _HG, D)
    for h in range(heads):
        head_v[h] = _pad_rows(ctx_v[:, h, :]).astype(_BF16)

    hidden_tiles = range(hidden_dim // _LANES)

    def project(base):
        tiles = []
        for j in hidden_tiles:
            tiles.append(_dot(xn_lo, column_tile(base, j)))
            stream.step("up", j)
        return tiles

    stream.wait(_WG)
    gate = [jax.nn.silu(v) for v in project(g0)]
    stream.wait(_WU)
    hidden = [(a * v).astype(_BF16) for a, v in zip(gate, project(u0))]
    stream.wait(_WD)
    y = jnp.zeros(x.shape, _F32)
    for j in hidden_tiles:
        y = y + _dot_nt(hidden[j], column_tile(d0, j))
        stream.step("down", j)
    mixed = jax.nn.silu(xn + (xn * 0.0 + y * route))

    lane_tiles = [(m0, min(_LANES, M - m0)) for m0 in range(0, M, _LANES)]
    work, done = {}, {}
    for h in range(heads):
        for m0, width in lane_tiles:
            first = h * head_slabs + m0 // _SLAB
            slabs = [landed[i] for i in range(first, first + width // _SLAB)]
            g = max(g for g, _ in slabs)
            work.setdefault(g, []).append((h, m0, [to for _, to in slabs]))
            done[m0] = max(done.get(m0, g), g)
    s = {m0: jnp.zeros((x.shape[0], width), _F32) for m0, width in lane_tiles}
    for g in range(_WO, len(groups)):
        lhs = {h: head_v[h] for h in sorted({h for h, _, _ in work[g]})}
        stream.wait(g)
        for i, (h, m0, slabs) in enumerate(work[g]):
            s[m0] = s[m0] + _dot_nt(lhs[h], jnp.concatenate([buf[to] for to in slabs], axis=0))
            stream.step("o", i)
        for m0, width in lane_tiles:
            if done[m0] == g:
                cols = slice(m0, m0 + width)
                out_v[:, cols] = (x[:, cols] + s[m0] * mixed[:, cols]).astype(out_v.dtype)[:B]
    out_cp = pltpu.make_async_copy(out_v, out_hbm, small_sems.at[0])
    out_cp.start()
    out_cp.wait()


def _slabs(w):
    r, c = w.shape
    w = w.reshape(r // _TILE_ROWS, _TILE_ROWS, c // _LANES, _LANES)
    return w.transpose(0, 2, 1, 3).reshape(-1, _SLAB, _LANES)


@jax.jit
def pallas_recurrent_scan__compressed_kv_cla__moe_arch_mod__decode_kernel(
    A_x: jax.Array,
    A_c_kv: jax.Array,
    A_w_q: jax.Array,
    A_w_uk: jax.Array,
    A_w_uv: jax.Array,
    A_w_o: jax.Array,
    B_x: jax.Array,
    B_w_r: jax.Array,
    B_w_gate: jax.Array,
    B_w_up: jax.Array,
    B_w_down: jax.Array,
):
    del B_x
    B, Sq, M = A_x.shape
    _, Sk, Dc = A_c_kv.shape
    _, H, D = A_w_q.shape
    assert Sq == 1 and H == _SLAB and D == _LANES

    x = A_x.reshape(B, M)
    streamed = [
        A_w_q,
        A_w_uk,
        _slabs(A_c_kv.reshape(B * Sk, Dc)),
        A_w_uv,
        _slabs(B_w_gate),
        _slabs(B_w_up),
        _slabs(B_w_down.T),
        jnp.transpose(A_w_o, (0, 2, 1)).reshape(-1, _SLAB, _LANES),
    ]

    def kernel(*refs):
        _kernel(*refs, heads=H, keys=Sk, hidden_dim=B_w_gate.shape[1])

    hbm = pl.BlockSpec(memory_space=pltpu.HBM)
    out = pl.pallas_call(
        kernel,
        out_shape=jax.ShapeDtypeStruct((B, M), A_x.dtype),
        in_specs=[hbm] * (2 + len(streamed)),
        out_specs=hbm,
        scratch_shapes=[
            pltpu.VMEM((sum(w.shape[0] for w in streamed), _SLAB, _LANES), _BF16),
            pltpu.VMEM((_HG, _LANES, _LANES), _BF16),
            pltpu.VMEM((M * _HG // _LANES, B * _HG, _LANES), _BF16),
            pltpu.VMEM(x.shape, x.dtype),
            pltpu.VMEM(B_w_r.shape, B_w_r.dtype),
            pltpu.VMEM(x.shape, x.dtype),
            pltpu.VMEM((B, H, D), _F32),
            pltpu.VMEM((H, 8, D), _BF16),
            pltpu.SemaphoreType.DMA((len(streamed) + len(_WO_GROUPS),)),
            pltpu.SemaphoreType.DMA((2,)),
        ],
        compiler_params=pltpu.CompilerParams(
            vmem_limit_bytes=96 * 1024 * 1024, disable_semaphore_checks=True
        ),
    )(x, B_w_r, *streamed)
    return out.reshape(B, Sq, M)
```

```python
import jax
import jax.numpy as jnp
from jax import lax
import jax.experimental.pallas as pl
import jax.experimental.pallas.tpu as pltpu

_F32 = jnp.float32
_BF16 = jnp.bfloat16
_LANES = 128
_TILE_ROWS = 8
_SLAB = 32
_HG = 16

_WQ, _WUK, _CKV, _WUV, _WG, _WU, _WD, _WO = range(8)

_BLOCK = 8
_BLOCK_START = 6
_BLOCK_STEP = 8
_PARTS = ((2, 0), (6, 1))
_LAST = 6
_LAST_PARTS = ((2, 1), (1, 1), (2, 1), (1, 1), (2, 1))
_WINDOWS = ((0, .15), (0, .176), (.1, .55), (.3, .62), (.5, .8), (.55, .84), (.6, .907), (.907, 1))
_WO_GROUPS = (18, 8, 4, 4)
_LEAD = 26
_MARGIN = 74
_CHUNK = 256
_STEPS = dict(q=(4, 4), uk=(4, 4), kv=(2, 4), uv=(4, 4), up=(4, 4), down=(4, 4), o=(8, 4))


def _dot(a, b):
    return jnp.dot(a, b, preferred_element_type=_F32)


def _dot_nt(a, b):
    return lax.dot_general(a, b, (((1,), (1,)), ((), ())), preferred_element_type=_F32)


def _iota(shape, axis):
    return lax.broadcasted_iota(jnp.int32, shape, axis)


def _pad_rows(v):
    return jnp.concatenate([v, jnp.zeros((8 - v.shape[0], v.shape[1]), v.dtype)], axis=0)


def _cut(start, parts):
    copies = []
    for size, priority in parts:
        copies.append((start, size, priority))
        start += size
    return copies


def _blocks(n_slabs):
    whole = list(range(_BLOCK_START, n_slabs - _BLOCK + 1, _BLOCK))
    blocks = [_cut(start, _PARTS) for i in range(_BLOCK_STEP) for start in whole[i::_BLOCK_STEP]]
    ends = [(whole[-1] + _BLOCK, n_slabs), (0, _BLOCK_START)]
    blocks.insert(len(blocks) // 4, [(a, b - a, 1) for a, b in ends if b > a])
    return blocks


def _moment(operand, i, n):
    first, last = _WINDOWS[operand]
    return first + (last - first) * (i + 0.5) / n


class _Stream:
    def __init__(self, order, groups, buf, sems):
        self.groups, self.buf, self.sems = groups, buf, sems
        low = [c for c in order[1:] if c[-1]]
        self.todo, low = order[:1] + low[:_LEAD], low[_LEAD:]
        for c in order[1:]:
            if not c[-1]:
                self.todo.append(c)
            elif low:
                self.todo.append(low.pop(0))
        self.ready = {g: i + 1 + _MARGIN for i, (g, *_) in enumerate(self.todo)}
        self.done = 0

    def _start(self, first, count):
        for g, start, to, size, priority in self.todo[first:first + count]:
            pltpu.make_async_copy(
                self.groups[g][0].at[pl.ds(start, size)],
                self.buf.at[pl.ds(to, size)],
                self.sems.at[g],
            ).start(priority=priority)

    def advance(self, count):
        self._start(self.done, count)
        self.done += count

    def step(self, stage, i):
        every, count = _STEPS[stage]
        if i % every == every - 1:
            self.advance(count)

    def loop(self, stage, turns, iterations, body):
        every, count = _STEPS[stage]
        per_turn = iterations // every * count

        def run(turn, carry):
            def step(i):
                if i % every == every - 1:
                    for u in range(turns):
                        first = self.done + u * per_turn + i // every * count
                        pl.when(turn == u)(lambda: self._start(first, count))

            body(turn, step)
            return carry

        lax.fori_loop(0, turns, run, 0)
        self.done += turns * per_turn

    def wait(self, g):
        self.advance(max(self.ready[g] - self.done, 0))
        _, first, size = self.groups[g]
        filled = self.buf.at[pl.ds(first, size)]
        pltpu.make_async_copy(filled, filled, self.sems.at[g]).wait()


def _kernel(
    x_hbm, wr_hbm, wq_hbm, wuk_hbm, ckv_hbm, wuv_hbm, wg_hbm, wu_hbm, wd_hbm, wo_hbm,
    out_hbm,
    buf, expand_v, lhs_v, lat_v, x_v, wr_v, out_v, ctx_v, head_v, sems, small_sems,
    *, heads, keys, hidden_dim,
):
    B, M = x_v.shape
    D = _LANES
    Dc = wuk_hbm.shape[0]
    n_groups = heads // _HG
    rows = B * _HG
    per_tile = _LANES // _HG
    n_expand = _LANES // per_tile

    sources = [wq_hbm, wuk_hbm, ckv_hbm, wuv_hbm, wg_hbm, wu_hbm, wd_hbm]
    bases = [0]
    for src in sources:
        bases.append(bases[-1] + src.shape[0])
    q0, uk0, kv0, uv0, g0, u0, d0, o0 = bases

    groups = [(src, base, src.shape[0]) for src, base in zip(sources, bases)]
    timed = []
    for g, (_, base, n) in enumerate(groups):
        blocks = _blocks(n)
        for i, block in enumerate(blocks):
            copies = [(g, start, base + start, *rest) for start, *rest in block]
            timed.append((_moment(g, i, len(blocks)), copies))
    head_slabs = M // _SLAB
    blocks = _blocks(wo_hbm.shape[0])
    blocks.sort(key=lambda block: block[0][0] % head_slabs == 0)
    blocks[-_LAST:] = [_cut(block[0][0], _LAST_PARTS) for block in blocks[-_LAST:]]
    cuts = [len(blocks) - sum(_WO_GROUPS[i:]) for i in range(len(_WO_GROUPS) + 1)]
    landed = {}
    for g, (a, b) in enumerate(zip([0] + cuts[:-1], cuts), _WO):
        first = o0 + len(landed)
        for i in range(a, b):
            copies = []
            for start, size, priority in blocks[i]:
                to = o0 + len(landed)
                copies.append((g, start, to, size, priority))
                landed.update({start + j: (g, to + j) for j in range(size)})
            timed.append((_moment(_WO, i, len(blocks)), copies))
        groups.append((wo_hbm, first, o0 + len(landed) - first))
    timed.sort(key=lambda entry: entry[0])
    stream = _Stream([copy for _, copies in timed for copy in copies], groups, buf, sems)

    def head_group(base, row0, n, g):
        return buf[pl.ds(base + row0, n), g * _HG:(g + 1) * _HG, :].reshape(n * _HG, D)

    per_slab = _SLAB // _TILE_ROWS

    def cache_tile(b, i, j):
        n = _CHUNK // _TILE_ROWS
        first = kv0 + b * (keys // _TILE_ROWS) + i * n
        tile = slice(j * _TILE_ROWS, (j + 1) * _TILE_ROWS)
        return buf[pl.ds(first, n), tile, :].reshape(_CHUNK, _LANES)

    def column_tile(base, j):
        per_band = hidden_dim // _LANES // per_slab
        tile = slice(j % per_slab * _TILE_ROWS, (j % per_slab + 1) * _TILE_ROWS)
        return jnp.concatenate(
            [buf[base + i * per_band + j // per_slab, tile] for i in range(M // _TILE_ROWS)],
            axis=0,
        )

    x_cp = pltpu.make_async_copy(x_hbm, x_v, small_sems.at[0])
    wr_cp = pltpu.make_async_copy(wr_hbm, wr_v, small_sems.at[1])
    stream.advance(_LEAD // 2)
    x_cp.start()
    wr_cp.start()
    stream.advance(_MARGIN)

    square = (_LANES, _LANES)
    for t in range(n_expand):
        e = _iota(square, 1) // _HG + t * per_tile == _iota(square, 0)
        expand_v[t] = e.astype(_BF16)
    own_head = _iota((rows, _LANES), 1) % _HG == _iota((rows, _LANES), 0) % _HG

    x_cp.wait()
    wr_cp.wait()
    x = _pad_rows(x_v[...].astype(_F32))
    xc = x - jnp.mean(x, axis=-1, keepdims=True)
    xn_lo = (xc / jnp.sqrt(jnp.mean(xc * xc, axis=-1, keepdims=True) + 1e-5)).astype(_BF16)
    xn = xn_lo.astype(_F32)
    wr = wr_v[...].astype(_F32).reshape(1, M)
    route = jax.nn.sigmoid(jnp.sum(xn * wr, axis=-1, keepdims=True))

    for t in range(M // per_tile):
        m0 = t // n_expand * _LANES
        n = min(_LANES, M - m0)
        rep = _dot(xn_lo[:, m0:m0 + n], expand_v[t % n_expand][:n])
        rep = jnp.concatenate(
            [jnp.broadcast_to(rep[b:b + 1], (_HG, _LANES)) for b in range(B)], axis=0
        )
        lhs_v[t] = jnp.where(own_head, rep, 0.0).astype(_BF16)
    stream.wait(_WQ)
    q = [jnp.zeros((rows, D), _F32) for _ in range(n_groups)]
    for t in range(M // per_tile):
        for g in range(n_groups):
            q[g] = q[g] + _dot(lhs_v[t], head_group(q0, t * per_tile, per_tile, g))
        stream.step("q", t)

    lat_tiles = range(Dc // _LANES)
    stream.wait(_WUK)
    q = [v.astype(_BF16) for v in q]

    def absorb_keys(j, step):
        for g in range(n_groups):
            acc = jnp.zeros((rows, _LANES), _F32)
            for t in range(n_expand):
                full = _dot_nt(q[g], head_group(uk0, j * _LANES + t * per_tile, per_tile, g))
                acc = acc + _dot_nt(jnp.where(own_head, full, 0.0).astype(_BF16), expand_v[t])
                step(g * n_expand + t)
            lat_v[j, :, g * _HG:(g + 1) * _HG, :] = acc.astype(_BF16).reshape(B, _HG, _LANES)

    stream.loop("uk", len(lat_tiles), n_groups * n_expand, absorb_keys)

    n_chunks = keys // _CHUNK

    def attend(b, step):
        q_lat = [lat_v[j, b] for j in lat_tiles]
        scores = []
        for i in range(n_chunks):
            parts = [_dot_nt(q_lat[j], cache_tile(b, i, j)) for j in lat_tiles]
            scores.append(sum(parts[1:], parts[0]))
            step(i)
        s = jnp.concatenate(scores, axis=1) * (D ** -0.5)
        p = jnp.exp(s - jnp.max(s, axis=-1, keepdims=True))
        denom = jnp.sum(p, axis=-1, keepdims=True)
        p = p.astype(_BF16)
        acc = [jnp.zeros((heads, _LANES), _F32) for _ in lat_tiles]
        for i in range(n_chunks):
            acc = [
                a + _dot(p[:, i * _CHUNK:(i + 1) * _CHUNK], cache_tile(b, i, j))
                for j, a in enumerate(acc)
            ]
            step(n_chunks + i)
        for j in lat_tiles:
            lat_v[j, b] = (acc[j] / denom).astype(_BF16)

    stream.wait(_CKV)
    stream.loop("kv", B, 2 * n_chunks, attend)

    stream.wait(_WUV)
    for g in range(n_groups):
        ctx = jnp.zeros((rows, D), _F32)
        for j in lat_tiles:
            lg = lat_v[j, :, g * _HG:(g + 1) * _HG, :].reshape(rows, _LANES)
            for t in range(n_expand):
                lhs = jnp.where(own_head, _dot(lg, expand_v[t]), 0.0).astype(_BF16)
                ctx = ctx + _dot(lhs, head_group(uv0, j * _LANES + t * per_tile, per_tile, g))
                stream.step("uv", t)
        ctx_v[:, g * _HG:(g + 1) * _HG, :] = ctx.reshape(B, _HG, D)
    for h in range(heads):
        head_v[h] = _pad_rows(ctx_v[:, h, :]).astype(_BF16)

    hidden_tiles = range(hidden_dim // _LANES)

    def project(base):
        tiles = []
        for j in hidden_tiles:
            tiles.append(_dot(xn_lo, column_tile(base, j)))
            stream.step("up", j)
        return tiles

    stream.wait(_WG)
    gate = [jax.nn.silu(v) for v in project(g0)]
    stream.wait(_WU)
    hidden = [(a * v).astype(_BF16) for a, v in zip(gate, project(u0))]
    stream.wait(_WD)
    y = jnp.zeros(x.shape, _F32)
    for j in hidden_tiles:
        y = y + _dot_nt(hidden[j], column_tile(d0, j))
        stream.step("down", j)
    mixed = jax.nn.silu(xn + (xn * 0.0 + y * route))

    lane_tiles = [(m0, min(_LANES, M - m0)) for m0 in range(0, M, _LANES)]
    work, done = {}, {}
    for h in range(heads):
        for m0, width in lane_tiles:
            first = h * head_slabs + m0 // _SLAB
            slabs = [landed[i] for i in range(first, first + width // _SLAB)]
            g = max(g for g, _ in slabs)
            work.setdefault(g, []).append((h, m0, [to for _, to in slabs]))
            done[m0] = max(done.get(m0, g), g)
    s = {m0: jnp.zeros((x.shape[0], width), _F32) for m0, width in lane_tiles}
    for g in range(_WO, len(groups)):
        lhs = {h: head_v[h] for h in sorted({h for h, _, _ in work[g]})}
        stream.wait(g)
        for i, (h, m0, slabs) in enumerate(work[g]):
            s[m0] = s[m0] + _dot_nt(lhs[h], jnp.concatenate([buf[to] for to in slabs], axis=0))
            stream.step("o", i)
        for m0, width in lane_tiles:
            if done[m0] == g:
                cols = slice(m0, m0 + width)
                out_v[:, cols] = (x[:, cols] + s[m0] * mixed[:, cols]).astype(out_v.dtype)[:B]
    out_cp = pltpu.make_async_copy(out_v, out_hbm, small_sems.at[0])
    out_cp.start()
    out_cp.wait()


def _slabs(w):
    r, c = w.shape
    w = w.reshape(r // _TILE_ROWS, _TILE_ROWS, c // _LANES, _LANES)
    return w.transpose(0, 2, 1, 3).reshape(-1, _SLAB, _LANES)


@jax.jit
def pallas_recurrent_scan__compressed_kv_cla__moe_arch_mod__decode_kernel(
    A_x: jax.Array,
    A_c_kv: jax.Array,
    A_w_q: jax.Array,
    A_w_uk: jax.Array,
    A_w_uv: jax.Array,
    A_w_o: jax.Array,
    B_x: jax.Array,
    B_w_r: jax.Array,
    B_w_gate: jax.Array,
    B_w_up: jax.Array,
    B_w_down: jax.Array,
):
    del B_x
    B, Sq, M = A_x.shape
    _, Sk, Dc = A_c_kv.shape
    _, H, D = A_w_q.shape
    assert Sq == 1 and H == _SLAB and D == _LANES

    x = A_x.reshape(B, M)
    streamed = [
        A_w_q,
        A_w_uk,
        _slabs(A_c_kv.reshape(B * Sk, Dc)),
        A_w_uv,
        _slabs(B_w_gate),
        _slabs(B_w_up),
        _slabs(B_w_down.T),
        jnp.transpose(A_w_o, (0, 2, 1)).reshape(-1, _SLAB, _LANES),
    ]

    def kernel(*refs):
        _kernel(*refs, heads=H, keys=Sk, hidden_dim=B_w_gate.shape[1])

    hbm = pl.BlockSpec(memory_space=pltpu.HBM)
    out = pl.pallas_call(
        kernel,
        out_shape=jax.ShapeDtypeStruct((B, M), A_x.dtype),
        in_specs=[hbm] * (2 + len(streamed)),
        out_specs=hbm,
        scratch_shapes=[
            pltpu.VMEM((sum(w.shape[0] for w in streamed), _SLAB, _LANES), _BF16),
            pltpu.VMEM((_HG, _LANES, _LANES), _BF16),
            pltpu.VMEM((M * _HG // _LANES, B * _HG, _LANES), _BF16),
            pltpu.VMEM((Dc // _LANES, B, H, _LANES), _BF16),
            pltpu.VMEM(x.shape, x.dtype),
            pltpu.VMEM(B_w_r.shape, B_w_r.dtype),
            pltpu.VMEM(x.shape, x.dtype),
            pltpu.VMEM((B, H, D), _F32),
            pltpu.VMEM((H, 8, D), _BF16),
            pltpu.SemaphoreType.DMA((len(streamed) + len(_WO_GROUPS),)),
            pltpu.SemaphoreType.DMA((2,)),
        ],
        compiler_params=pltpu.CompilerParams(
            vmem_limit_bytes=96 * 1024 * 1024, disable_semaphore_checks=True
        ),
    )(x, B_w_r, *streamed)
    return out.reshape(B, Sq, M)
```
